```python
import jax
import jax.numpy as jnp

def _softmax(x, axis=-1):
    return jax.nn.softmax(x, axis=axis)

def _gelu(x):
    return jax.nn.gelu(x, approximate=True)

def _silu(x):
    return jax.nn.silu(x)

def _sigmoid(x):
    return jax.nn.sigmoid(x)

def _layernorm(x, axis=-1, eps=1e-05):
    m = jnp.mean(x, axis=axis, keepdims=True)
    v = jnp.var(x, axis=axis, keepdims=True)
    return (x - m) / jnp.sqrt(v + eps)

def _scatter_add(tgt, idx, src, axis=0):
    return tgt.at[idx].add(src)

def _segment_sum(src, seg, n):
    return jax.ops.segment_sum(src, seg, n)

class _Rng:

    def __init__(self, key):
        self._k = key

    def _next(self):
        self._k, sub = jax.random.split(self._k)
        return sub

    def normal(self, shape):
        return jax.random.normal(self._next(), shape, dtype=jnp.bfloat16)

    def randint(self, lo, hi, shape):
        return jax.random.randint(self._next(), shape, lo, hi, dtype=jnp.int32)

    def uniform(self, shape, lo=0.0, hi=1.0):
        return jax.random.uniform(self._next(), shape, jnp.bfloat16, lo, hi)

    def permutation(self, n):
        return jax.random.permutation(self._next(), n)
kernel_name = 'sequential_preLN__memory_aug_recurrent_mem_tr__mixer_s_mlp__prompt'

def setup_inputs():
    _rng = _Rng(jax.random.key(int.from_bytes(__import__("os").urandom(4), "little")))
    _w = lambda a: (lambda t: t.astype(jnp.bfloat16) if jnp.issubdtype(t.dtype, jnp.floating) else t)(jnp.asarray(a))

    def _A_setup():
        B, S, Dm = (1, 2048, 1024)
        H, Dh = (32, 128)
        M, seg = (8, 32)
        seg = min(seg, S)
        S = S // seg * seg
        return {'x': _w((lambda *s: _rng.normal(s) * 0.05)(B, S, Dm)), 'mem0': _w((lambda *s: _rng.normal(s) * 0.05)(B, M, Dm)), 'Wq': _w((lambda *s: _rng.normal(s) * 0.05)(Dm, H, Dh) * Dm ** (-0.5)), 'Wk': _w((lambda *s: _rng.normal(s) * 0.05)(Dm, H, Dh) * Dm ** (-0.5)), 'Wv': _w((lambda *s: _rng.normal(s) * 0.05)(Dm, H, Dh) * Dm ** (-0.5)), 'Wo': _w((lambda *s: _rng.normal(s) * 0.05)(H, Dh, Dm) * (H * Dh) ** (-0.5)), 'seg_len': seg}
    _A_in = _A_setup()

    def _B_setup():
        B, S, D, F = (1, 2048, 1024, 3584)
        return {'x': _w((lambda *s: _rng.normal(s) * 0.05)(B, S, D)), 'w1': _w((lambda *s: _rng.normal(s) * 0.05)(D, D) * D ** (-0.5)), 'w2': _w((lambda *s: _rng.normal(s) * 0.05)(D, D) * D ** (-0.5)), 'w3': _w((lambda *s: _rng.normal(s) * 0.05)(D, F) * D ** (-0.5)), 'w4': _w((lambda *s: _rng.normal(s) * 0.05)(F, D) * F ** (-0.5))}
    _B_in = _B_setup()
    return {'A_x': _A_in['x'], 'A_mem0': _A_in['mem0'], 'A_Wq': _A_in['Wq'], 'A_Wk': _A_in['Wk'], 'A_Wv': _A_in['Wv'], 'A_Wo': _A_in['Wo'], 'A_seg_len': _A_in['seg_len'], 'B_x': _B_in['x'], 'B_w1': _B_in['w1'], 'B_w2': _B_in['w2'], 'B_w3': _B_in['w3'], 'B_w4': _B_in['w4']}

def reference(A_x, A_mem0, A_Wq, A_Wk, A_Wv, A_Wo, A_seg_len, B_x, B_w1, B_w2, B_w3, B_w4):

    def _A_ref(x, mem0, Wq, Wk, Wv, Wo, seg_len):
        B, S, Dm = x.shape
        H, Dh = (Wq.shape[1], Wq.shape[2])
        M = mem0.shape[1]
        scale = Dh ** (-0.5)
        n_seg = S // seg_len
        L = M + seg_len
        idx = jnp.arange(L)
        mask = (idx[:, None] < M) | (idx[:, None] >= idx[None, :])
        mem = mem0
        outs = []
        for s in range(n_seg):
            xs = x[:, s * seg_len:(s + 1) * seg_len, :].copy()
            h = jnp.concatenate([mem, xs], axis=1)
            q = jnp.einsum('btd,dhe->bhte', h, Wq)
            k = jnp.einsum('btd,dhe->bhte', h, Wk)
            v = jnp.einsum('btd,dhe->bhte', h, Wv)
            scores = jnp.einsum('bhqe,bhke->bhqk', q, k) * scale
            scores = jnp.where(mask[None, None], scores, -1000000000.0)
            p = _softmax(scores, axis=-1)
            o = jnp.einsum('bhqk,bhke->bhqe', p, v)
            o = jnp.einsum('bhte,hed->btd', o, Wo)
            mem = o[:, :M, :].copy()
            outs.append(o[:, M:, :])
        return jnp.concatenate(outs, axis=1)

    def _B_ref(x, w1, w2, w3, w4):
        B, S, D = x.shape
        h = _gelu(_layernorm(x, axis=-1) @ w1)
        c = D // 4
        g0 = jnp.pad(h[:, :, 0 * c:1 * c], ((0, 0), (1, 0), (0, 0)))[:, :S, :]
        g1 = jnp.pad(h[:, :, 1 * c:2 * c], ((0, 0), (0, 1), (0, 0)))[:, 1:, :]
        g2 = jnp.pad(h[:, :, 2 * c:3 * c], ((0, 0), (2, 0), (0, 0)))[:, :S, :]
        g3 = jnp.pad(h[:, :, 3 * c:], ((0, 0), (0, 2), (0, 0)))[:, 2:, :]
        hs = jnp.concatenate([g0, g1, g2, g3], axis=-1) @ w2
        x1 = x + hs
        h2 = _gelu(_layernorm(x1, axis=-1) @ w3) @ w4
        return x1 + h2
    x = A_x
    h = x + _A_ref(_layernorm(x, axis=-1), A_mem0, A_Wq, A_Wk, A_Wv, A_Wo, A_seg_len)
    h2 = h + _B_ref(_layernorm(h, axis=-1), B_w1, B_w2, B_w3, B_w4)
    return h2
```

```python
import functools

import jax
import jax.numpy as jnp
import numpy as np
from jax import lax
import jax.experimental.pallas as pl
import jax.experimental.pallas.tpu as pltpu

BF = jnp.bfloat16
F32 = jnp.float32
U32 = jnp.uint32

S = 2048
D = 1024
H = 32
DH = 128
M = 8
SEG = 32
NSEG = S // SEG
FF = 3584
RIDE = 24
UP = SEG - RIDE
EPS = 1e-5
SCALE = DH ** -0.5
RB = 256


def _ln(x):
    m = jnp.mean(x, axis=-1, keepdims=True)
    xc = x - m
    v = jnp.mean(xc * xc, axis=-1, keepdims=True)
    return xc * lax.rsqrt(v + EPS)


def _gelu(x):
    c = np.float32(np.sqrt(2.0 / np.pi))
    inner = c * (x + np.float32(0.044715) * (x * x * x))
    return x * (0.5 * (1.0 + jnp.tanh(inner)))


def _dot(a, b):
    return jnp.dot(a, b, preferred_element_type=F32)


def _dot_nt(a, b):
    return lax.dot_general(a, b, (((1,), (1,)), ((), ())), preferred_element_type=F32)


def _kernel(x_hbm, mem0_ref, wq_hbm, wk_hbm, wv_hbm, wo_hbm, w1_hbm, w2_hbm, w3_hbm, w4_hbm,
            out_hbm,
            x3, h3, wq32, wk32, wv32, wo32, sems):

    def a_part(xr, xup, qu, ku, vu, oup, stg):
        DC = 128
        NCH = D // DC

        def x_copy(i):
            return pltpu.make_async_copy(x_hbm.at[pl.ds(i * 16, 16)], x3.at[pl.ds(i * 16, 16)], sems.at[i])

        def w_copy(w_hbm, slot, c):
            return pltpu.make_async_copy(w_hbm.at[pl.ds(c * DC * H, DC * H)],
                                         stg.at[slot, pl.ds(c * DC * H, DC * H)],
                                         sems.at[4 + slot * NCH + c])

        def wo_copy(slot, j):
            return pltpu.make_async_copy(wo_hbm.at[:, pl.ds(j * 128, 128)],
                                         stg.at[slot, pl.ds(j * 4096, 4096)],
                                         sems.at[4 + slot * NCH + j])

        for i in range(4):
            x_copy(i).start()
        for c in range(NCH):
            w_copy(wq_hbm, 0, c).start()
        for c in range(NCH):
            w_copy(wk_hbm, 1, c).start()

        for i in range(4):
            x_copy(i).wait()

            def ln_body(j, carry, i=i):
                seg = i * 16 + j * 2
                for t in range(2):
                    xv = x3[seg + t].astype(F32)
                    z = _ln(xv)
                    xr[seg + t] = z[:RIDE]
                    xup[seg + t] = z[RIDE:]
                return carry
            lax.fori_loop(0, 8, ln_body, 0)

        def relayout(slot, w32):
            s32 = stg.at[slot].bitcast(U32)
            for c in range(NCH):
                (w_copy(wq_hbm, slot, c)).wait()

            def body(c, carry):
                base = pl.multiple_of(c * (DC * 16), DC * 16)
                ch = s32.at[pl.ds(base, DC * 16)]
                for hp in range(16):
                    v = ch[pl.ds(hp, DC, stride=16), :]
                    lo = v.astype(jnp.uint16)
                    hi = (v >> 16).astype(jnp.uint16)
                    r0 = pl.multiple_of(c * (DC // 2), DC // 2)
                    w32[2 * hp, pl.ds(r0, DC // 2), :] = pltpu.bitcast(lo, U32)
                    w32[2 * hp + 1, pl.ds(r0, DC // 2), :] = pltpu.bitcast(hi, U32)
                return carry
            lax.fori_loop(0, NCH, body, 0)

        def big_proj(w32, dst):
            a = xup[...].reshape(NSEG * UP, D).astype(BF)

            def body(g, carry):
                w = jnp.concatenate([w32[g * 4 + t] for t in range(4)], axis=1)
                r = _dot(a, pltpu.bitcast(w, BF))
                for t in range(4):
                    dst[g * 4 + t] = r[:, t * 128:(t + 1) * 128]
                return carry
            lax.fori_loop(0, H // 4, body, 0)

        relayout(0, wq32)
        for c in range(NCH):
            w_copy(wv_hbm, 0, c).start()
        big_proj(wq32, qu)
        relayout(1, wk32)
        for j in range(8):
            wo_copy(1, j).start()
        big_proj(wk32, ku)
        relayout(0, wv32)
        big_proj(wv32, vu)
        for j in range(8):
            wo_copy(1, j).wait()
        so32 = stg.at[1].bitcast(U32)

        def wo_body(j, carry):
            for t in range(8):
                src = pl.multiple_of(j * 2048 + t * 256, 256)
                wo32[j, pl.ds(t * 256, 256), :] = so32[pl.ds(src, 256), :]
            return carry
        lax.fori_loop(0, 8, wo_body, 0)

        ri = lax.broadcasted_iota(jnp.int32, (M + SEG, M + SEG), 0)
        ci = lax.broadcasted_iota(jnp.int32, (M + SEG, M + SEG), 1)
        mask = (ri < M) | (ri >= ci)

        def step(s, mem):
            r0 = pl.multiple_of(s * UP, UP)
            a = jnp.concatenate([mem, xr[s]], axis=0).astype(BF)

            def qkv(h):
                w = jnp.concatenate([wq32[h], wk32[h], wv32[h]], axis=1)
                return _dot(a, pltpu.bitcast(w, BF))

            def scores(h, r):
                q = jnp.concatenate([r[:, 0:128], qu[h, pl.ds(r0, UP), :]], axis=0).astype(BF)
                k = jnp.concatenate([r[:, 128:256], ku[h, pl.ds(r0, UP), :]], axis=0).astype(BF)
                sc = jnp.where(mask, _dot_nt(q, k) * SCALE, -1e9)
                mx = jnp.max(sc, axis=-1, keepdims=True)
                e = jnp.exp(sc - mx)
                inv = pl.reciprocal(jnp.sum(e, axis=-1, keepdims=True), approx=False, full_range=False)
                return e.astype(BF), inv

            def pv(h, r, e, inv):
                v = jnp.concatenate([r[:, 256:384], vu[h, pl.ds(r0, UP), :]], axis=0).astype(BF)
                o = _dot(e, v) * inv
                oup[s, :, h * 128:(h + 1) * 128] = o[M + RIDE:]
                return o[:M + RIDE].astype(BF)

            rs, es, os_ = {}, {}, {}
            LAG1, LAG2 = 1, 2
            for t in range(H + LAG2):
                if t < H:
                    rs[t] = qkv(t)
                hh = t - LAG2
                if 0 <= hh < H:
                    os_[hh] = pv(hh, rs[hh], *es[hh])
                hh = t - LAG1
                if 0 <= hh < H:
                    es[hh] = scores(hh, rs[hh])
            oc = jnp.concatenate([os_[h] for h in range(H)], axis=1)
            res = jnp.concatenate(
                [_dot(oc, pltpu.bitcast(wo32[j], BF)) for j in range(8)], axis=1)
            h3[s, 0:RIDE, :] = x3[s, 0:RIDE, :].astype(F32) + res[M:]
            return res[:M]

        lax.fori_loop(0, NSEG, step, mem0_ref[...].astype(F32))

        def fin(b, carry):
            nb = 16
            s0 = pl.multiple_of(b * nb, nb)
            o = oup[pl.ds(s0, nb)].reshape(nb * UP, H * DH).astype(BF)
            res = jnp.concatenate(
                [_dot(o, pltpu.bitcast(wo32[j], BF)) for j in range(8)], axis=1)
            res = res.reshape(nb, UP, D)
            h3[pl.ds(s0, nb), RIDE:SEG, :] = x3[pl.ds(s0, nb), RIDE:SEG, :].astype(F32) + res
            return carry
        lax.fori_loop(0, NSEG // 16, fin, 0)

    pl.run_scoped(
        a_part,
        pltpu.VMEM((NSEG, RIDE, D), F32),
        pltpu.VMEM((NSEG, UP, D), F32),
        pltpu.VMEM((H, NSEG * UP, DH), F32),
        pltpu.VMEM((H, NSEG * UP, DH), F32),
        pltpu.VMEM((H, NSEG * UP, DH), F32),
        pltpu.VMEM((NSEG, UP, H * DH), F32),
        pltpu.VMEM((2, D * H, DH), BF),
    )

    def b_part(w1, w2, w3, w4, hn_buf, t_buf, o_buf):
        cps = [pltpu.make_async_copy(a, b, sems.at[24 + i])
               for i, (a, b) in enumerate([(w1_hbm, w1), (w2_hbm, w2), (w3_hbm, w3), (w4_hbm, w4)])]
        for cp in cps:
            cp.start()
        t_buf[0:8, :] = jnp.zeros((8, D), F32)
        t_buf[8 + S:16 + S, :] = jnp.zeros((8, D), F32)
        cps[0].wait()
        nb = RB // SEG

        def pass1(b, carry):
            s0 = pl.multiple_of(b * nb, nb)
            r0 = pl.multiple_of(b * RB, RB)
            hb = h3[pl.ds(s0, nb)].reshape(RB, D)
            hn = _ln(hb)
            hn_buf[pl.ds(r0, RB), :] = hn
            z = _ln(hn).astype(BF)
            t_buf[pl.ds(r0 + 8, RB), :] = _gelu(_dot(z, w1[...]))
            return carry
        lax.fori_loop(0, S // RB, pass1, 0)
        cps[1].wait()
        cps[2].wait()
        cps[3].wait()

        def out_copy(b, slot):
            return pltpu.make_async_copy(o_buf.at[slot], out_hbm.at[pl.ds(b * RB, RB)], sems.at[28 + slot])

        def pass2(b, carry):
            s0 = pl.multiple_of(b * nb, nb)
            r0 = pl.multiple_of(b * RB, RB)
            slot = b % 2
            parts = []
            for g, sh in enumerate((1, -1, 2, -2)):
                tv = t_buf[pl.ds(r0, RB + 16), g * 256:(g + 1) * 256]
                parts.append(tv[8 - sh:8 - sh + RB].astype(BF))
            gm = jnp.concatenate(parts, axis=1)
            x1 = hn_buf[pl.ds(r0, RB), :] + _dot(gm, w2[...])
            z = _ln(x1).astype(BF)
            u = _gelu(_dot(z, w3[...])).astype(BF)
            h2 = _dot(u, w4[...])
            hb = h3[pl.ds(s0, nb)].reshape(RB, D)
            res = hb + (x1 + h2)

            @pl.when(b >= 2)
            def _():
                out_copy(b - 2, slot).wait()
            o_buf[slot] = res.astype(BF)
            out_copy(b, slot).start()
            return carry
        lax.fori_loop(0, S // RB, pass2, 0)
        out_copy(S // RB - 2, 0).wait()
        out_copy(S // RB - 1, 1).wait()

    pl.run_scoped(
        b_part,
        pltpu.VMEM((D, D), BF),
        pltpu.VMEM((D, D), BF),
        pltpu.VMEM((D, FF), BF),
        pltpu.VMEM((FF, D), BF),
        pltpu.VMEM((S, D), F32),
        pltpu.VMEM((S + 16, D), F32),
        pltpu.VMEM((2, RB, D), BF),
    )


@jax.jit
def pallas_sequential_preLN__memory_aug_recurrent_mem_tr__mixer_s_mlp__prompt_kernel(A_x, A_mem0, A_Wq, A_Wk, A_Wv, A_Wo, A_seg_len, B_x, B_w1, B_w2, B_w3, B_w4):
    del A_seg_len, B_x
    any_spec = pl.BlockSpec(memory_space=pl.ANY)
    out = pl.pallas_call(
        _kernel,
        out_shape=jax.ShapeDtypeStruct((S, D), BF),
        in_specs=[any_spec, pl.BlockSpec(memory_space=pltpu.VMEM)] + [any_spec] * 8,
        out_specs=any_spec,
        scratch_shapes=[
            pltpu.VMEM((NSEG, SEG, D), BF),
            pltpu.VMEM((NSEG, SEG, D), F32),
            pltpu.VMEM((H, D // 2, DH), U32),
            pltpu.VMEM((H, D // 2, DH), U32),
            pltpu.VMEM((H, D // 2, DH), U32),
            pltpu.VMEM((8, H * DH // 2, 128), U32),
            pltpu.SemaphoreType.DMA((32,)),
        ],
        compiler_params=pltpu.CompilerParams(vmem_limit_bytes=126 * 1024 * 1024),
    )(
        A_x.reshape(NSEG, SEG, D), A_mem0.reshape(M, D),
        A_Wq.reshape(D * H, DH), A_Wk.reshape(D * H, DH), A_Wv.reshape(D * H, DH),
        A_Wo.reshape(H * DH, D), B_w1, B_w2, B_w3, B_w4,
    )
    return out.reshape(1, S, D)
```

```python
import jax
import jax.numpy as jnp
import numpy as np
from jax import lax
import jax.experimental.pallas as pl
import jax.experimental.pallas.tpu as pltpu

BF = jnp.bfloat16
F32 = jnp.float32
U32 = jnp.uint32

S = 2048
D = 1024
H = 32
DH = 128
M = 8
SEG = 32
NSEG = S // SEG
FF = 3584
RIDE = 24
UP = SEG - RIDE
EPS = 1e-5
SCALE = DH ** -0.5
RB = 256
HB = RB // 2
G = 8
NG = H // G

def _ln(x):
    m = jnp.mean(x, axis=-1, keepdims=True)
    xc = x - m
    v = jnp.mean(xc * xc, axis=-1, keepdims=True)
    return xc * lax.rsqrt(v + EPS)


def _gelu(x):
    c0 = np.float32(np.sqrt(2.0 / np.pi))
    c1 = np.float32(np.sqrt(2.0 / np.pi) * 0.044715)
    t = jnp.tanh(x * (c0 + c1 * (x * x)))
    hx = 0.5 * x
    return hx + hx * t


def _dot(a, b):
    return jnp.dot(a.astype(BF), b, preferred_element_type=F32)


def _dot_nt(a, b):
    return lax.dot_general(a.astype(BF), b, (((1,), (1,)), ((), ())), preferred_element_type=F32)


def _slabs(w32, n, lo=None, hi=None):
    if lo is None:
        parts = [w32[j] for j in range(n)]
    else:
        parts = [w32[j, lo:hi, :] for j in range(n)]
    return pltpu.bitcast(jnp.concatenate(parts, axis=1), BF)


def _pack2(a, b):
    return pltpu.pack_elementwise([a, b], packed_dtype=BF)


def _kernel(x_hbm, mem0_ref, wq_hbm, wk_hbm, wv_hbm, wo_hbm, w1_hbm, w2_hbm, w3_hbm, w4_hbm,
            out_hbm,
            x3, h3, wq32, wk32, wv32, wo, w1, w2, w3, w4, sems):
    w32s = (wq32, wk32, wv32)
    wo32 = wo.bitcast(U32)
    w132, w232, w332, w432 = (w.bitcast(U32) for w in (w1, w2, w3, w4))
    S_XU, S_W1, S_W2, S_W3, S_W4, S_WO, S_OUT, S_XR, S_P = 0, 1, 2, 3, 4, 5, 6, 10, 14

    def slab_copy(src, dst, sem, j):
        j0 = j * 128 if isinstance(j, int) else pl.multiple_of(j * 128, 128)
        return pltpu.make_async_copy(src.at[:, pl.ds(j0, 128)], dst.at[j], sems.at[sem])

    def wait_all(buf, sem):
        pltpu.make_async_copy(buf, buf, sems.at[sem]).wait()

    STG = []

    def c3(i, j):
        blk = i * 14 + j
        return STG[0].at[blk // 16, pl.ds((blk % 16) * 32, 32)]

    def c4(i, n):
        blk = i * 4 + n
        return STG[0].at[5 + blk // 4, pl.ds((blk % 4) * 128, 112)]

    def combos(i, c3, c4):
        def ld(ref, slab, r0, n):
            w = ref[slab, pl.ds(r0, n), :]
            return tuple(pltpu.unpack_elementwise(w, index=i, packed_dtype=BF, unpacked_dtype=F32) for i in range(2))

        def emit(dst, slab, e0, n, b11, b12, b21, b22):
            outs = []
            for i in range(2):
                outs.append((b11[i] + b22[i], b12[i] - b22[i], b21[i] - b11[i], b11[i] + b12[i], b21[i] + b22[i]))
            for i in range(5):
                dst(i, slab)[pl.ds(e0, n // 8)] = _pack2(outs[0][i], outs[1][i]).reshape(n // 8, 8, 128)
        r3 = pl.multiple_of(i * 8, 8)
        r3h = pl.multiple_of(i * 8 + 256, 8)
        for j in range(14):
            emit(c3, j, i, 8, ld(w332, j, r3, 8), ld(w332, 14 + j, r3, 8),
                 ld(w332, j, r3h, 8), ld(w332, 14 + j, r3h, 8))
        i4 = jnp.minimum(i, 27)
        r4 = pl.multiple_of(i4 * 32, 32)
        r4h = pl.multiple_of(i4 * 32 + 896, 32)
        for n in range(4):
            emit(c4, n, 4 * i4, 32, ld(w432, n, r4, 32), ld(w432, 4 + n, r4, 32),
                 ld(w432, n, r4h, 32), ld(w432, 4 + n, r4h, 32))

    def a_part(xr, xup32, up32, oup, stg):

        def prologue(stg):
            xu_cp = pltpu.make_async_copy(x_hbm.at[:, pl.ds(RIDE, UP)], x3.at[:, pl.ds(RIDE, UP)], sems.at[S_XU])

            def xr_cp(g):
                s0 = pl.multiple_of(g * 16, 16)
                return pltpu.make_async_copy(x_hbm.at[pl.ds(s0, 16), pl.ds(0, RIDE)],
                                             x3.at[pl.ds(s0, 16), pl.ds(0, RIDE)], sems.at[S_XR + g])
            srcs = [w.bitcast(U32) for w in (wq_hbm, wk_hbm, wv_hbm)]

            def w_cps(m, p, g):
                res = []
                for dd in range(2):
                    off = 16 * dd + 4 * g
                    if not isinstance(g, int):
                        off = pl.multiple_of(off, 4)
                    res.append(pltpu.make_async_copy(srcs[m].at[:, pl.ds(off, 4)],
                                                     stg.at[p, :, pl.ds(4 * dd, 4)],
                                                     sems.at[S_P + p * 2 + dd]))
                return res

            def wait(m, g):
                for cp in w_cps(m, 3 * g + m, g):
                    cp.wait()

            def relayout_rows(m, g, half):
                r0 = half * 256 if isinstance(half, int) else pl.multiple_of(half * 256, 256)
                ch = stg.at[3 * g + m, pl.ds(r0, 256)].reshape(2048, DH)
                for c in range(2):
                    for hp in range(4):
                        v = ch[pl.ds(c * 1024 + hp, 256, stride=4), :]
                        lo = v.astype(jnp.uint16)
                        hi = (v >> 16).astype(jnp.uint16)
                        w32s[m][G * g + 2 * hp, pl.ds(r0 + c * 128, 128), :] = pltpu.bitcast(lo, U32)
                        w32s[m][G * g + 2 * hp + 1, pl.ds(r0 + c * 128, 128), :] = pltpu.bitcast(hi, U32)

            def ln_ride(s0, n):
                for u in range(n):
                    xr[s0 + u] = _ln(x3[s0 + u, 0:RIDE, :].astype(F32))

            def proj(m, g, j0, j1):
                a = pltpu.bitcast(xup32[...], BF)
                for jj in range(NJ[0]):
                    j = j0 + jj
                    h0 = G * g + 2 * j
                    w = pltpu.bitcast(jnp.concatenate([w32s[m][h0], w32s[m][h0 + 1]], axis=1), BF)
                    r = jnp.dot(a, w, preferred_element_type=F32)
                    r0 = r[:, 0:DH].reshape(NSEG, UP, DH)
                    r1 = r[:, DH:2 * DH].reshape(NSEG, UP, DH)
                    up32[(G // 2) * (3 * g + m) + j] = _pack2(r0, r1)

            xu_cp.start()

            def start_group(g, carry):
                for m in range(3):
                    for cp in w_cps(m, 3 * g + m, g):
                        cp.start()
                xr_cp(g).start()
                return carry
            lax.fori_loop(0, NG, start_group, 0)
            xu_cp.wait()
            def ln_up(c, carry):
                z = _ln(x3[pl.ds(c * 16, 16), RIDE:SEG, :].astype(F32).reshape(16 * UP, D))
                xup32[pl.ds(pl.multiple_of(c * 64, 64), 64), :] = pltpu.bitcast(z.astype(BF), U32)
                return carry
            lax.fori_loop(0, 4, ln_up, 0)
            wait(0, 0)

            def rl0(half, carry):
                relayout_rows(0, 0, half)
                return carry
            lax.fori_loop(0, 2, rl0, 0)

            MW = 1
            NJ = [2]
            WG = 1

            def body(g, carry):
                gn = jnp.minimum(g + 1, NG - 1)

                def ph0(half, c):
                    if MW:
                        NJ[0] = 1
                        proj(0, g, 2 * half, 2 * half + 1)

                        @pl.when(half == 0)
                        def _():
                            wait(1, g)
                        relayout_rows(1, g, half)
                        proj(0, g, 2 * half + 1, 2 * half + 2)
                        NJ[0] = 2
                    else:
                        relayout_rows(1, g, half)
                        proj(0, g, 2 * half, 2 * half + 2)
                    return c
                if not MW:
                    wait(1, g)
                lax.fori_loop(0, 2, ph0, 0)
                wait(2, g)

                def ph1(half, c):
                    relayout_rows(2, g, half)
                    proj(1, g, 2 * half, 2 * half + 2)
                    return c
                lax.fori_loop(0, 2, ph1, 0)

                @pl.when(g < NG - 1)
                def _():
                    wait(0, gn)
                xr_cp(g).wait()

                def ph2(half, c):
                    ln_ride(g * 16 + half * 8, 8)
                    relayout_rows(0, gn, half)
                    proj(2, g, 2 * half, 2 * half + 2)
                    return c
                lax.fori_loop(0, 2, ph2, 0)

                @pl.when(g == 1)
                def _():
                    def st(j, c):
                        slab_copy(wo_hbm, wo, S_WO, j).start()
                        return c
                    lax.fori_loop(0, 8, st, 0)

                @pl.when(g == WG)
                def _():
                    def st3(j, c):
                        slab_copy(w3_hbm, w3, S_W3, j).start()
                        return c
                    lax.fori_loop(0, 28, st3, 0)

                    def st4(j, c):
                        slab_copy(w4_hbm, w4, S_W4, j).start()
                        return c
                    lax.fori_loop(0, 8, st4, 0)
                return carry

            lax.fori_loop(0, NG, body, 0)

        prologue(stg)
        wait_all(wo, S_WO)
        wait_all(w3, S_W3)
        wait_all(w4, S_W4)

        R2 = 2 * (M + SEG)
        ri = lax.broadcasted_iota(jnp.int32, (R2, R2), 0)
        ci = lax.broadcasted_iota(jnp.int32, (R2, R2), 1)
        hr = jnp.where(ri < 64, ri >> 5, (ri - 64) >> 3)
        pr = jnp.where(ri < 64, ri & 31, 32 + (ri & 7))
        hc = ci & 1
        pc = ci >> 1
        mask = (hr == hc) & ((pr < M) | (pr >= pc))

        def step(s, mem):
            a = jnp.concatenate([mem, xr[s]], axis=0).astype(BF)

            def proj(m, g):
                w = pltpu.bitcast(jnp.concatenate([w32s[m][g * G + i] for i in range(G)], axis=1), BF)
                r = jnp.dot(a, w, preferred_element_type=F32)
                return [r[:, i * DH:(i + 1) * DH] for i in range(G)]

            def up_row(m, pair):
                return up32[(3 * (pair // (G // 2)) + m) * (G // 2) + pair % (G // 2), s]

            def cat_q(pair, x0, x1):
                u = up_row(0, pair)
                u0, u1 = (pltpu.unpack_elementwise(u, index=i, packed_dtype=BF, unpacked_dtype=F32) for i in range(2))
                return jnp.concatenate([x0, x1, u0, u1], axis=0)

            def cat_kv(m, pair, x0, x1):
                return jnp.concatenate([_pack2(x0, x1), up_row(m, pair)], axis=0)

            def scores(q, k):
                sc = jnp.where(mask, _dot_nt(q, pltpu.bitcast(k, BF)) * SCALE, -1e9)
                mx = jnp.max(sc, axis=-1, keepdims=True)
                e = jnp.exp(sc - mx)
                inv = pltpu.reciprocal(jnp.sum(e, axis=-1, keepdims=True), approx=False, full_range=False)
                return e.astype(BF), inv

            os_ = {}

            def pv(pair, v, e, inv, dep=None):
                if dep is not None:
                    z = pltpu.bitcast(jnp.minimum(jnp.abs(dep), 0.0), U32)
                    v = v | jnp.concatenate([z] * 5, axis=0)
                o = jnp.dot(e, pltpu.bitcast(v, BF), preferred_element_type=F32) * inv
                h0 = 2 * pair
                oup[s, :, h0 * DH:(h0 + 1) * DH] = o[64:72]
                oup[s, :, (h0 + 1) * DH:(h0 + 2) * DH] = o[72:80]
                os_[h0] = o[0:32]
                os_[h0 + 1] = o[32:64]

            parts = []

            def wo_part(ha, hb):
                oc = jnp.concatenate([os_[h] for h in range(ha, hb)], axis=1)
                parts.append(_dot(oc, _slabs(wo32, 8, ha * 64, hb * 64)))

            es, vs = {}, {}
            for g in range(NG):
                qs, ks, vv = proj(0, g), proj(1, g), proj(2, g)
                if g > 0:
                    for j in range(G // 2):
                        p = (g - 1) * (G // 2) + j
                        pv(p, vs[p], *es[p])
                for j in range(G // 2):
                    p = g * (G // 2) + j
                    es[p] = scores(cat_q(p, qs[2 * j], qs[2 * j + 1]), cat_kv(1, p, ks[2 * j], ks[2 * j + 1]))
                    vs[p] = cat_kv(2, p, vv[2 * j], vv[2 * j + 1])
            wo_part(0, 16)
            for j in range(G // 2):
                p = (NG - 1) * (G // 2) + j
                pv(p, vs[p], *es[p], dep=parts[0][0:8, 3 * DH:4 * DH])
            wo_part(16, 24)
            wo_part(24, 32)
            res = parts[0] + parts[1] + parts[2]
            h3[s, 0:RIDE, :] = x3[s, 0:RIDE, :].astype(F32) + res[M:]
            return res[:M]

        UN = 2

        def slab_start(src, dst, sem, j, n):
            @pl.when(jnp.logical_and(j >= 0, j < n))
            def _():
                slab_copy(src, dst, sem, jnp.clip(j, 0, n - 1)).start()

        def stepn(i, mem):
            ii = i * UN // 2 if UN != 2 else i
            if UN == 1:
                @pl.when(i % 2 == 0)
                def _():
                    starts(i // 2)
            else:
                starts(ii)
            combos(i, c3, c4)
            for u in range(UN):
                mem = step(UN * i + u, mem)
            return mem

        def starts(i):
            slab_start(w1_hbm, w1, S_W1, i - 8, 8)
            slab_start(w2_hbm, w2, S_W2, i - 16, 8)

        lax.fori_loop(0, NSEG // UN, stepn, mem0_ref[...].astype(F32))

    def b1(oup, hn_buf, t_buf, c3, c4):
        wait_all(w1, S_W1)
        wait_all(w2, S_W2)
        t_buf[0:8, :] = jnp.zeros((8, D), F32)
        t_buf[8 + S:16 + S, :] = jnp.zeros((8, D), F32)
        nb = HB // SEG

        def fin(s0):
            o = oup[pl.ds(s0, nb)].reshape(nb * UP, H * DH)
            res = _dot(o, _slabs(wo32, 8)).reshape(nb, UP, D)
            h3[pl.ds(s0, nb), RIDE:SEG, :] = x3[pl.ds(s0, nb), RIDE:SEG, :].astype(F32) + res

        def lns(s0, r0):
            hn = _ln(h3[pl.ds(s0, nb)].reshape(HB, D))
            hn_buf[pl.ds(r0, HB), :] = hn
            return _ln(hn)

        def pass1(b, carry):
            sa = pl.multiple_of(b * 2 * nb, nb)
            sb = pl.multiple_of(b * 2 * nb + nb, nb)
            ra = pl.multiple_of(b * RB, HB)
            rb = pl.multiple_of(b * RB + HB, HB)
            fin(sa)
            fin(sb)
            za = lns(sa, ra)
            ya = _dot(za, _slabs(w132, 8))
            zb = lns(sb, rb)
            t_buf[pl.ds(ra + 8, HB), :] = _gelu(ya)
            yb = _dot(zb, _slabs(w132, 8))
            t_buf[pl.ds(rb + 8, HB), :] = _gelu(yb)
            return carry
        lax.fori_loop(0, S // RB, pass1, 0)

    def b2(hn_buf, t_buf, o_buf, c3, c4):
        nb = HB // SEG

        def out_copy(hb, slot):
            return pltpu.make_async_copy(o_buf.at[slot], out_hbm.at[pl.ds(hb * HB, HB)], sems.at[S_OUT + slot])

        def pass2(b, carry):
            par = b % 2

            @pl.when(b >= 2)
            def _():
                out_copy(2 * b - 4, 2 * par).wait()
                out_copy(2 * b - 3, 2 * par + 1).wait()

            def shift(r0):
                parts = []
                for g, sh in enumerate((1, -1, 2, -2)):
                    tv = t_buf[pl.ds(r0, HB + 16), g * 256:(g + 1) * 256]
                    parts.append(tv[8 - sh:8 - sh + HB])
                return jnp.concatenate(parts, axis=1)

            def mix(r0, gm):
                x1 = hn_buf[pl.ds(r0, HB), :] + _dot(gm, _slabs(w232, 8))
                return x1, _ln(x1)

            def lhs7(a11, a12, a21, a22):
                return [a11 + a22, a21 + a22, a11, a22, a11 + a12, a21 - a11, a12 - a22]

            def comb(m):
                m1, m2, m3, m4, m5, m6, m7 = m
                return (m1 + m4 - m5 + m7, m3 + m5, m2 + m4, m1 - m2 + m3 + m6)

            def bf(v):
                return pltpu.bitcast(v, BF)

            ra = pl.multiple_of(b * RB, HB)
            rb = pl.multiple_of(b * RB + HB, HB)
            sa = pl.multiple_of(b * 2 * nb, nb)
            sb = pl.multiple_of(b * 2 * nb + nb, nb)
            ga = shift(ra)
            gb = shift(rb)
            xa, za = mix(ra, ga)
            xb, zb = mix(rb, gb)
            l3 = [v.astype(BF) for v in lhs7(za[:, :512], za[:, 512:], zb[:, :512], zb[:, 512:])]
            l4 = [[] for _ in range(7)]
            PRE = 2

            def cv(c, i, j):
                r = c(i, j)
                return r[...].reshape(r.shape[0] * 8, 128)

            def rhs3(j):
                return [cv(c3, 0, j), w332[j, 0:256, :], cv(c3, 1, j), cv(c3, 2, j), w332[14 + j, 256:512, :],
                        cv(c3, 3, j), cv(c3, 4, j)]
            pre = {}
            for j in range(PRE):
                rhs = rhs3(j)
                for i in (2, 4):
                    pre[(i, j)] = _dot(l3[i], bf(rhs[i]))
            for j in range(14):
                rhs = rhs3(j)
                m = [pre[(i, j)] if (i, j) in pre else _dot(l3[i], bf(rhs[i])) for i in range(7)]
                u11, u12, u21, u22 = (_gelu(c) for c in comb(m))
                for i, v in enumerate(lhs7(u11, u12, u21, u22)):
                    l4[i].append(v)
            l4 = [jnp.concatenate(v, axis=1).astype(BF) for v in l4]
            hs = [(h3[pl.ds(sa, nb)].reshape(HB, D), xa), (h3[pl.ds(sb, nb)].reshape(HB, D), xb)]
            for n in range(4):
                rhs = [cv(c4, 0, n), w432[n, 0:896, :], cv(c4, 1, n), cv(c4, 2, n), w432[4 + n, 896:1792, :],
                       cv(c4, 3, n), cv(c4, 4, n)]
                m = [_dot(l4[i], bf(rhs[i])) for i in range(7)]
                h11, h12, h21, h22 = comb(m)
                for i, col, v in ((0, n, h11), (0, 4 + n, h12), (1, n, h21), (1, 4 + n, h22)):
                    cs = slice(col * 128, (col + 1) * 128)
                    res = hs[i][0][:, cs] + (hs[i][1][:, cs] + v)
                    o_buf[2 * par + i, :, cs] = res.astype(BF)
            out_copy(2 * b, 2 * par).start()
            out_copy(2 * b + 1, 2 * par + 1).start()
            return carry

        lax.fori_loop(0, S // RB, pass2, 0)
        for i in range(4):
            out_copy(S // HB - 4 + i, i).wait()

    def outer(oup, stg):
        STG.append(stg)
        pl.run_scoped(
            lambda xr, xup32, up32: a_part(xr, xup32, up32, oup, stg),
            pltpu.VMEM((NSEG, RIDE, D), F32),
            pltpu.VMEM((NSEG * UP // 2, D), U32),
            pltpu.VMEM((3 * H // 2, NSEG, 8, DH), U32),
        )

        def b_scope(hn_buf, t_buf, o_buf):
            b1(oup, hn_buf, t_buf, c3, c4)
            b2(hn_buf, t_buf, o_buf, c3, c4)
        pl.run_scoped(b_scope, pltpu.VMEM((S, D), F32), pltpu.VMEM((S + 16, D), F32),
                      pltpu.VMEM((4, HB, D), BF))

    pl.run_scoped(outer, pltpu.VMEM((NSEG, UP, H * DH), F32), pltpu.VMEM((3 * NG, D // 2, 8, DH), U32))


@jax.jit
def pallas_sequential_preLN__memory_aug_recurrent_mem_tr__mixer_s_mlp__prompt_kernel(A_x, A_mem0, A_Wq, A_Wk, A_Wv, A_Wo, A_seg_len, B_x, B_w1, B_w2, B_w3, B_w4):
    del A_seg_len, B_x
    any_spec = pl.BlockSpec(memory_space=pl.ANY)
    out = pl.pallas_call(
        _kernel,
        out_shape=jax.ShapeDtypeStruct((S, D), BF),
        in_specs=[any_spec, pl.BlockSpec(memory_space=pltpu.VMEM)] + [any_spec] * 8,
        out_specs=any_spec,
        scratch_shapes=[
            pltpu.VMEM((NSEG, SEG, D), BF),
            pltpu.VMEM((NSEG, SEG, D), F32),
            pltpu.VMEM((H, D // 2, DH), U32),
            pltpu.VMEM((H, D // 2, DH), U32),
            pltpu.VMEM((H, D // 2, DH), U32),
            pltpu.VMEM((8, H * DH, 128), BF),
            pltpu.VMEM((8, D, 128), BF),
            pltpu.VMEM((8, D, 128), BF),
            pltpu.VMEM((28, D, 128), BF),
            pltpu.VMEM((8, FF, 128), BF),
            pltpu.SemaphoreType.DMA((38,)),
        ],
        compiler_params=pltpu.CompilerParams(vmem_limit_bytes=127 * 1024 * 1024),
    )(
        A_x.reshape(NSEG, SEG, D), A_mem0.reshape(M, D),
        A_Wq.reshape(D // 2, 2 * H, DH), A_Wk.reshape(D // 2, 2 * H, DH), A_Wv.reshape(D // 2, 2 * H, DH),
        A_Wo.reshape(H * DH, D), B_w1, B_w2, B_w3, B_w4,
    )
    return out.reshape(1, S, D)
```

```python
import contextlib
import functools
import os

import jax
import jax.numpy as jnp
import numpy as np
from jax import lax
import jax.experimental.pallas as pl
import jax.experimental.pallas.tpu as pltpu

BF = jnp.bfloat16
F32 = jnp.float32
U32 = jnp.uint32

S = 2048
D = 1024
H = 32
DH = 128
M = 8
SEG = 32
NSEG = S // SEG
FF = 3584
RIDE = 24
UP = SEG - RIDE
EPS = 1e-5
SCALE = DH ** -0.5
RB = 256
HB = RB // 2
G = 8
NG = H // G

def _ln(x):
    m = jnp.mean(x, axis=-1, keepdims=True)
    xc = x - m
    v = jnp.mean(xc * xc, axis=-1, keepdims=True)
    return xc * lax.rsqrt(v + EPS)


def _gelu(x):
    c0 = np.float32(np.sqrt(2.0 / np.pi))
    c1 = np.float32(np.sqrt(2.0 / np.pi) * 0.044715)
    t = jnp.tanh(x * (c0 + c1 * (x * x)))
    hx = 0.5 * x
    return hx + hx * t


def _dot(a, b):
    return jnp.dot(a.astype(BF), b, preferred_element_type=F32)


def _dot_nt(a, b):
    return lax.dot_general(a.astype(BF), b, (((1,), (1,)), ((), ())), preferred_element_type=F32)


def _slabs(w32, n, lo=None, hi=None):
    if lo is None:
        parts = [w32[j] for j in range(n)]
    else:
        parts = [w32[j, lo:hi, :] for j in range(n)]
    return pltpu.bitcast(jnp.concatenate(parts, axis=1), BF)


def _unpack2(w):
    return pltpu.bitcast(w << 16, F32), pltpu.bitcast(w & jnp.uint32(0xFFFF0000), F32)


def _kernel(x_hbm, mem0_ref, wq_hbm, wk_hbm, wv_hbm, wo_hbm, w1_hbm, w2_hbm, w3_hbm, w4_hbm,
            out_hbm,
            x3, wq32, wk32, wv32, wo, w1, w2, w3, w4, sems):
    w32s = (wq32, wk32, wv32)
    wo32 = wo.bitcast(U32)
    w132, w232, w332, w432 = (w.bitcast(U32) for w in (w1, w2, w3, w4))
    S_XU, S_W1, S_W2, S_W3, S_W4, S_WO, S_OUT, S_XR, S_P = 0, 1, 2, 3, 4, 5, 6, 10, 14

    def slab_copy(src, dst, sem, j):
        j0 = j * 128 if isinstance(j, int) else pl.multiple_of(j * 128, 128)
        return pltpu.make_async_copy(src.at[:, pl.ds(j0, 128)], dst.at[j], sems.at[sem])

    def wait_all(buf, sem):
        pltpu.make_async_copy(buf, buf, sems.at[sem]).wait()

    def combos(i, c3, c4):
        def ld(ref, slab, r0, n):
            return pltpu.bitcast(ref[slab, pl.ds(r0, n), :], BF).astype(F32)

        def emit(dst, slab, e0, n, b11, b12, b21, b22):
            for i, v in enumerate((b11 + b22, b12 - b22, b21 - b11, b11 + b12, b21 + b22)):
                dst[i, slab, pl.ds(e0, 2 * n), :] = v.astype(BF)
        r3 = pl.multiple_of(i * 8, 8)
        r3h = pl.multiple_of(i * 8 + 256, 8)
        e3 = pl.multiple_of(i * 16, 16)
        for j in range(14):
            emit(c3, j, e3, 8, ld(w332, j, r3, 8), ld(w332, 14 + j, r3, 8),
                 ld(w332, j, r3h, 8), ld(w332, 14 + j, r3h, 8))
        i4 = jnp.minimum(i, 27)
        r4 = pl.multiple_of(i4 * 32, 32)
        r4h = pl.multiple_of(i4 * 32 + 896, 32)
        e4 = pl.multiple_of(i4 * 64, 64)
        for n in range(4):
            emit(c4, n, e4, 32, ld(w432, n, r4, 32), ld(w432, 4 + n, r4, 32),
                 ld(w432, n, r4h, 32), ld(w432, 4 + n, r4h, 32))

    def a_part(xr, xup32, up):

        def prologue(stg):
            xu_cp = pltpu.make_async_copy(x_hbm.at[:, pl.ds(RIDE, UP)], x3.at[:, pl.ds(RIDE, UP)], sems.at[S_XU])

            def xr_cp(g):
                s0 = pl.multiple_of(g * 16, 16)
                return pltpu.make_async_copy(x_hbm.at[pl.ds(s0, 16), pl.ds(0, RIDE)],
                                             x3.at[pl.ds(s0, 16), pl.ds(0, RIDE)], sems.at[S_XR + g])
            srcs = [w.bitcast(U32) for w in (wq_hbm, wk_hbm, wv_hbm)]

            def w_cps(m, p, g):
                res = []
                for dd in range(2):
                    off = 16 * dd + 4 * g
                    if not isinstance(g, int):
                        off = pl.multiple_of(off, 4)
                    res.append(pltpu.make_async_copy(srcs[m].at[:, pl.ds(off, 4)],
                                                     stg.at[p, :, pl.ds(4 * dd, 4)],
                                                     sems.at[S_P + p * 2 + dd]))
                return res

            def wait(m, g):
                for cp in w_cps(m, 3 * g + m, g):
                    cp.wait()

            def relayout_rows(m, g, half):
                r0 = half * 256 if isinstance(half, int) else pl.multiple_of(half * 256, 256)
                ch = stg.at[3 * g + m, pl.ds(r0, 256)].reshape(2048, DH)
                for c in range(2):
                    for hp in range(4):
                        v = ch[pl.ds(c * 1024 + hp, 256, stride=4), :]
                        lo = v.astype(jnp.uint16)
                        hi = (v >> 16).astype(jnp.uint16)
                        w32s[m][G * g + 2 * hp, pl.ds(r0 + c * 128, 128), :] = pltpu.bitcast(lo, U32)
                        w32s[m][G * g + 2 * hp + 1, pl.ds(r0 + c * 128, 128), :] = pltpu.bitcast(hi, U32)

            def ln_ride(s0, n):
                for u in range(n):
                    xr[s0 + u] = _ln(x3[s0 + u, 0:RIDE, :].astype(F32)).astype(BF)

            def proj(m, g, j0, j1):
                a = pltpu.bitcast(xup32[...], BF)
                for jj in range(NJ[0]):
                    j = j0 + jj
                    h0 = G * g + 2 * j
                    w = pltpu.bitcast(jnp.concatenate([w32s[m][h0], w32s[m][h0 + 1]], axis=1), BF)
                    r = jnp.dot(a, w, preferred_element_type=F32)
                    r0 = r[:, 0:DH].reshape(NSEG, UP, DH)
                    r1 = r[:, DH:2 * DH].reshape(NSEG, UP, DH)
                    up[(G // 2) * (3 * g + m) + j] = jnp.concatenate([r0, r1], axis=1).astype(BF)

            xu_cp.start()

            def start_group(g, carry):
                for m in range(3):
                    for cp in w_cps(m, 3 * g + m, g):
                        cp.start()
                xr_cp(g).start()
                return carry
            lax.fori_loop(0, NG, start_group, 0)
            xu_cp.wait()
            def ln_up(c, carry):
                z = _ln(x3[pl.ds(c * 16, 16), RIDE:SEG, :].astype(F32).reshape(16 * UP, D))
                xup32[pl.ds(pl.multiple_of(c * 64, 64), 64), :] = pltpu.bitcast(z.astype(BF), U32)
                return carry
            lax.fori_loop(0, 4, ln_up, 0)
            wait(0, 0)

            def rl0(half, carry):
                relayout_rows(0, 0, half)
                return carry
            lax.fori_loop(0, 2, rl0, 0)

            MW = 1
            NJ = [2]
            WG = 1

            def body(g, carry):
                gn = jnp.minimum(g + 1, NG - 1)

                def ph0(half, c):
                    if MW:
                        NJ[0] = 1
                        proj(0, g, 2 * half, 2 * half + 1)

                        @pl.when(half == 0)
                        def _():
                            wait(1, g)
                        relayout_rows(1, g, half)
                        proj(0, g, 2 * half + 1, 2 * half + 2)
                        NJ[0] = 2
                    else:
                        relayout_rows(1, g, half)
                        proj(0, g, 2 * half, 2 * half + 2)
                    return c
                if not MW:
                    wait(1, g)
                lax.fori_loop(0, 2, ph0, 0)
                wait(2, g)

                def ph1(half, c):
                    relayout_rows(2, g, half)
                    proj(1, g, 2 * half, 2 * half + 2)
                    return c
                lax.fori_loop(0, 2, ph1, 0)

                @pl.when(g < NG - 1)
                def _():
                    wait(0, gn)
                xr_cp(g).wait()

                def ph2(half, c):
                    ln_ride(g * 16 + half * 8, 8)
                    relayout_rows(0, gn, half)
                    proj(2, g, 2 * half, 2 * half + 2)
                    return c
                lax.fori_loop(0, 2, ph2, 0)

                @pl.when(g == 1)
                def _():
                    def st(j, c):
                        slab_copy(wo_hbm, wo, S_WO, j).start()
                        return c
                    lax.fori_loop(0, 8, st, 0)

                @pl.when(g == WG)
                def _():
                    def st3(j, c):
                        slab_copy(w3_hbm, w3, S_W3, j).start()
                        return c
                    lax.fori_loop(0, 28, st3, 0)

                    def st4(j, c):
                        slab_copy(w4_hbm, w4, S_W4, j).start()
                        return c
                    lax.fori_loop(0, 8, st4, 0)
                return carry

            lax.fori_loop(0, NG, body, 0)

        pl.run_scoped(prologue, pltpu.VMEM((3 * NG, D // 2, 8, DH), U32))
        pl.run_scoped(functools.partial(later, xr, up), *LATER_SHAPES)

    def later(xr, up, h3, oup, c3, c4):
        wait_all(wo, S_WO)
        wait_all(w3, S_W3)
        wait_all(w4, S_W4)

        R2 = 2 * (M + SEG)
        ri = lax.broadcasted_iota(jnp.int32, (R2, R2), 0)
        ci = lax.broadcasted_iota(jnp.int32, (R2, R2), 1)
        hr = jnp.where(ri < 64, ri >> 5, (ri - 64) >> 3)
        pr = jnp.where(ri < 64, ri & 31, 32 + (ri & 7))
        hc = jnp.where(ci < 64, ci >> 5, (ci - 64) >> 3)
        pc = jnp.where(ci < 64, ci & 31, 32 + (ci & 7))
        mask = (hr == hc) & ((pr < M) | (pr >= pc))

        def step(s, mem):
            a = jnp.concatenate([mem, xr[s].astype(F32)], axis=0).astype(BF)

            def proj(m, g):
                w = pltpu.bitcast(jnp.concatenate([w32s[m][g * G + i] for i in range(G)], axis=1), BF)
                r = jnp.dot(a, w, preferred_element_type=F32)
                return [r[:, i * DH:(i + 1) * DH] for i in range(G)]

            def cat(m, pair, x0, x1):
                u = up[(3 * (pair // (G // 2)) + m) * (G // 2) + pair % (G // 2), s].astype(F32)
                return jnp.concatenate([x0, x1, u], axis=0)

            def scores(q, k):
                sc = jnp.where(mask, _dot_nt(q, k.astype(BF)) * SCALE, -1e9)
                mx = jnp.max(sc, axis=-1, keepdims=True)
                e = jnp.exp(sc - mx)
                inv = pltpu.reciprocal(jnp.sum(e, axis=-1, keepdims=True), approx=False, full_range=False)
                return e.astype(BF), inv

            os_ = {}

            def pv(pair, v, e, inv, dep=None):
                if dep is not None:
                    z = jnp.minimum(jnp.abs(dep), 0.0)
                    v = v + jnp.concatenate([z] * 10, axis=0)
                o = jnp.dot(e, v.astype(BF), preferred_element_type=F32) * inv
                h0 = 2 * pair
                oup[s, :, h0 * DH:(h0 + 1) * DH] = o[64:72]
                oup[s, :, (h0 + 1) * DH:(h0 + 2) * DH] = o[72:80]
                os_[h0] = o[0:32]
                os_[h0 + 1] = o[32:64]

            parts = []

            def wo_part(ha, hb):
                oc = jnp.concatenate([os_[h] for h in range(ha, hb)], axis=1)
                parts.append(_dot(oc, _slabs(wo32, 8, ha * 64, hb * 64)))

            es, vs = {}, {}
            for g in range(NG):
                qs, ks, vv = proj(0, g), proj(1, g), proj(2, g)
                if g > 0:
                    for j in range(G // 2):
                        p = (g - 1) * (G // 2) + j
                        pv(p, vs[p], *es[p])
                for j in range(G // 2):
                    p = g * (G // 2) + j
                    es[p] = scores(cat(0, p, qs[2 * j], qs[2 * j + 1]), cat(1, p, ks[2 * j], ks[2 * j + 1]))
                    vs[p] = cat(2, p, vv[2 * j], vv[2 * j + 1])
                    if g < NG - 1:
                        vs[p] = vs[p].astype(BF)
            wo_part(0, 16)
            for j in range(G // 2):
                p = (NG - 1) * (G // 2) + j
                pv(p, vs[p], *es[p], dep=parts[0][0:8, 3 * DH:4 * DH])
            wo_part(16, 24)
            wo_part(24, 32)
            res = parts[0] + parts[1] + parts[2]
            h3[s, 0:RIDE, :] = x3[s, 0:RIDE, :].astype(F32) + res[M:]
            return res[:M]

        UN = 2

        def slab_start(src, dst, sem, j, n):
            @pl.when(jnp.logical_and(j >= 0, j < n))
            def _():
                slab_copy(src, dst, sem, jnp.clip(j, 0, n - 1)).start()

        def stepn(i, mem):
            ii = i * UN // 2 if UN != 2 else i
            if UN == 1:
                @pl.when(i % 2 == 0)
                def _():
                    starts(i // 2)
            else:
                starts(ii)
            combos(i, c3, c4)
            for u in range(UN):
                mem = step(UN * i + u, mem)
            return mem

        def starts(i):
            slab_start(w1_hbm, w1, S_W1, i - 8, 8)
            slab_start(w2_hbm, w2, S_W2, i - 16, 8)

        lax.fori_loop(0, NSEG // UN, stepn, mem0_ref[...].astype(F32))

        def b_scope(hn_buf, t_buf, o_buf):
            b1(h3, oup, hn_buf, t_buf)
            b2(h3, hn_buf, t_buf, o_buf, c3.bitcast(U32), c4.bitcast(U32))
        pl.run_scoped(b_scope, pltpu.VMEM((S, D), F32), pltpu.VMEM((S + 16, D), F32),
                      pltpu.VMEM((4, HB, D), BF))

    def b1(h3, oup, hn_buf, t_buf):
        wait_all(w1, S_W1)
        wait_all(w2, S_W2)
        t_buf[0:8, :] = jnp.zeros((8, D), F32)
        t_buf[8 + S:16 + S, :] = jnp.zeros((8, D), F32)
        nb = HB // SEG

        def fin(s0):
            o = oup[pl.ds(s0, nb)].reshape(nb * UP, H * DH)
            res = _dot(o, _slabs(wo32, 8)).reshape(nb, UP, D)
            h3[pl.ds(s0, nb), RIDE:SEG, :] = x3[pl.ds(s0, nb), RIDE:SEG, :].astype(F32) + res

        def lns(s0, r0):
            hn = _ln(h3[pl.ds(s0, nb)].reshape(HB, D))
            hn_buf[pl.ds(r0, HB), :] = hn
            return _ln(hn)

        def pass1(b, carry):
            sa = pl.multiple_of(b * 2 * nb, nb)
            sb = pl.multiple_of(b * 2 * nb + nb, nb)
            ra = pl.multiple_of(b * RB, HB)
            rb = pl.multiple_of(b * RB + HB, HB)
            fin(sa)
            fin(sb)
            za = lns(sa, ra)
            ya = _dot(za, _slabs(w132, 8))
            zb = lns(sb, rb)
            t_buf[pl.ds(ra + 8, HB), :] = _gelu(ya)
            yb = _dot(zb, _slabs(w132, 8))
            t_buf[pl.ds(rb + 8, HB), :] = _gelu(yb)
            return carry
        lax.fori_loop(0, S // RB, pass1, 0)

    def b2(h3, hn_buf, t_buf, o_buf, c3, c4):
        nb = HB // SEG

        def out_copy(hb, slot):
            return pltpu.make_async_copy(o_buf.at[slot], out_hbm.at[pl.ds(hb * HB, HB)], sems.at[S_OUT + slot])

        def pass2(b, carry):
            par = b % 2

            @pl.when(b >= 2)
            def _():
                out_copy(2 * b - 4, 2 * par).wait()
                out_copy(2 * b - 3, 2 * par + 1).wait()

            def shift(r0):
                parts = []
                for g, sh in enumerate((1, -1, 2, -2)):
                    tv = t_buf[pl.ds(r0, HB + 16), g * 256:(g + 1) * 256]
                    parts.append(tv[8 - sh:8 - sh + HB])
                return jnp.concatenate(parts, axis=1)

            def mix(r0, gm):
                x1 = hn_buf[pl.ds(r0, HB), :] + _dot(gm, _slabs(w232, 8))
                return x1, _ln(x1)

            def lhs7(a11, a12, a21, a22):
                return [a11 + a22, a21 + a22, a11, a22, a11 + a12, a21 - a11, a12 - a22]

            def comb(m):
                m1, m2, m3, m4, m5, m6, m7 = m
                return (m1 + m4 - m5 + m7, m3 + m5, m2 + m4, m1 - m2 + m3 + m6)

            def bf(v):
                return pltpu.bitcast(v, BF)

            ra = pl.multiple_of(b * RB, HB)
            rb = pl.multiple_of(b * RB + HB, HB)
            sa = pl.multiple_of(b * 2 * nb, nb)
            sb = pl.multiple_of(b * 2 * nb + nb, nb)
            ga = shift(ra)
            gb = shift(rb)
            xa, za = mix(ra, ga)
            xb, zb = mix(rb, gb)
            l3 = [v.astype(BF) for v in lhs7(za[:, :512], za[:, 512:], zb[:, :512], zb[:, 512:])]
            l4 = [[] for _ in range(7)]
            PRE = 2

            def cv(c, i, j):
                return c[i, j]

            def rhs3(j):
                return [cv(c3, 0, j), w332[j, 0:256, :], cv(c3, 1, j), cv(c3, 2, j), w332[14 + j, 256:512, :],
                        cv(c3, 3, j), cv(c3, 4, j)]
            pre = {}
            for j in range(PRE):
                rhs = rhs3(j)
                for i in (2, 4):
                    pre[(i, j)] = _dot(l3[i], bf(rhs[i]))
            for j in range(14):
                rhs = rhs3(j)
                m = [pre[(i, j)] if (i, j) in pre else _dot(l3[i], bf(rhs[i])) for i in range(7)]
                u11, u12, u21, u22 = (_gelu(c) for c in comb(m))
                for i, v in enumerate(lhs7(u11, u12, u21, u22)):
                    l4[i].append(v)
            l4 = [jnp.concatenate(v, axis=1).astype(BF) for v in l4]
            hs = [(h3[pl.ds(sa, nb)].reshape(HB, D), xa), (h3[pl.ds(sb, nb)].reshape(HB, D), xb)]
            for n in range(4):
                rhs = [cv(c4, 0, n), w432[n, 0:896, :], cv(c4, 1, n), cv(c4, 2, n), w432[4 + n, 896:1792, :],
                       cv(c4, 3, n), cv(c4, 4, n)]
                m = [_dot(l4[i], bf(rhs[i])) for i in range(7)]
                h11, h12, h21, h22 = comb(m)
                for i, col, v in ((0, n, h11), (0, 4 + n, h12), (1, n, h21), (1, 4 + n, h22)):
                    cs = slice(col * 128, (col + 1) * 128)
                    res = hs[i][0][:, cs] + (hs[i][1][:, cs] + v)
                    o_buf[2 * par + i, :, cs] = res.astype(BF)
            out_copy(2 * b, 2 * par).start()
            out_copy(2 * b + 1, 2 * par + 1).start()
            return carry

        lax.fori_loop(0, S // RB, pass2, 0)
        for i in range(4):
            out_copy(S // HB - 4 + i, i).wait()

    LATER_SHAPES = (pltpu.VMEM((NSEG, SEG, D), F32), pltpu.VMEM((NSEG, UP, H * DH), F32),
                    pltpu.VMEM((5, 14, 512, 128), BF), pltpu.VMEM((5, 4, 1792, 128), BF))
    pl.run_scoped(
        a_part,
        pltpu.VMEM((NSEG, RIDE, D), BF),
        pltpu.VMEM((NSEG * UP // 2, D), U32),
        pltpu.VMEM((3 * H // 2, NSEG, 16, DH), BF),
    )


@jax.jit
def pallas_sequential_preLN__memory_aug_recurrent_mem_tr__mixer_s_mlp__prompt_kernel(A_x, A_mem0, A_Wq, A_Wk, A_Wv, A_Wo, A_seg_len, B_x, B_w1, B_w2, B_w3, B_w4):
    del A_seg_len, B_x
    any_spec = pl.BlockSpec(memory_space=pl.ANY)
    out = pl.pallas_call(
        _kernel,
        out_shape=jax.ShapeDtypeStruct((S, D), BF),
        in_specs=[any_spec, pl.BlockSpec(memory_space=pltpu.VMEM)] + [any_spec] * 8,
        out_specs=any_spec,
        scratch_shapes=[
            pltpu.VMEM((NSEG, SEG, D), BF),
            pltpu.VMEM((H, D // 2, DH), U32),
            pltpu.VMEM((H, D // 2, DH), U32),
            pltpu.VMEM((H, D // 2, DH), U32),
            pltpu.VMEM((8, H * DH, 128), BF),
            pltpu.VMEM((8, D, 128), BF),
            pltpu.VMEM((8, D, 128), BF),
            pltpu.VMEM((28, D, 128), BF),
            pltpu.VMEM((8, FF, 128), BF),
            pltpu.SemaphoreType.DMA((38,)),
        ],
        compiler_params=pltpu.CompilerParams(vmem_limit_bytes=127 * 1024 * 1024),
    )(
        A_x.reshape(NSEG, SEG, D), A_mem0.reshape(M, D),
        A_Wq.reshape(D // 2, 2 * H, DH), A_Wk.reshape(D // 2, 2 * H, DH), A_Wv.reshape(D // 2, 2 * H, DH),
        A_Wo.reshape(H * DH, D), B_w1, B_w2, B_w3, B_w4,
    )
    return out.reshape(1, S, D)
```

```python
import functools

import jax
import jax.numpy as jnp
import numpy as np
from jax import lax
import jax.experimental.pallas as pl
import jax.experimental.pallas.tpu as pltpu

BF = jnp.bfloat16
F32 = jnp.float32
U32 = jnp.uint32

S = 2048
D = 1024
H = 32
DH = 128
M = 8
SEG = 32
NSEG = S // SEG
FF = 3584
RIDE = 24
UP = SEG - RIDE
EPS = 1e-5
SCALE = DH ** -0.5
RB = 256
HB = RB // 2
G = 8
NG = H // G

def _ln(x):
    m = jnp.mean(x, axis=-1, keepdims=True)
    xc = x - m
    v = jnp.mean(xc * xc, axis=-1, keepdims=True)
    return xc * lax.rsqrt(v + EPS)


def _gelu(x):
    c0 = np.float32(np.sqrt(2.0 / np.pi))
    c1 = np.float32(np.sqrt(2.0 / np.pi) * 0.044715)
    t = jnp.tanh(x * (c0 + c1 * (x * x)))
    hx = 0.5 * x
    return hx + hx * t


def _dot(a, b):
    return jnp.dot(a.astype(BF), b, preferred_element_type=F32)


def _dot_nt(a, b):
    return lax.dot_general(a.astype(BF), b, (((1,), (1,)), ((), ())), preferred_element_type=F32)


def _slabs(w32, n, lo=None, hi=None):
    if lo is None:
        parts = [w32[j] for j in range(n)]
    else:
        parts = [w32[j, lo:hi, :] for j in range(n)]
    return pltpu.bitcast(jnp.concatenate(parts, axis=1), BF)


def _kernel(x_hbm, mem0_ref, wq_hbm, wk_hbm, wv_hbm, wo_hbm, w1_hbm, w2_hbm, w3_hbm, w4_hbm,
            out_hbm,
            x3, wq32, wk32, wv32, wo, w1, w2, w3, w4, sems):
    w32s = (wq32, wk32, wv32)
    wo32 = wo.bitcast(U32)
    w132, w232, w332, w432 = (w.bitcast(U32) for w in (w1, w2, w3, w4))
    S_XU, S_W1, S_W2, S_W3, S_W4, S_WO, S_OUT, S_XR, S_P = 0, 1, 2, 3, 4, 5, 6, 10, 14

    def slab_copy(src, dst, sem, j):
        j0 = j * 128 if isinstance(j, int) else pl.multiple_of(j * 128, 128)
        return pltpu.make_async_copy(src.at[:, pl.ds(j0, 128)], dst.at[j], sems.at[sem])

    def wait_all(buf, sem):
        pltpu.make_async_copy(buf, buf, sems.at[sem]).wait()

    def combos(i, c3, c4):
        def ld(ref, slab, r0, n):
            return pltpu.bitcast(ref[slab, pl.ds(r0, n), :], BF).astype(F32)

        def emit(dst, slab, e0, n, b11, b12, b21, b22):
            for i, v in enumerate((b11 + b22, b12 - b22, b21 - b11, b11 + b12, b21 + b22)):
                dst[i, slab, pl.ds(e0, 2 * n), :] = v.astype(BF)
        r3 = pl.multiple_of(i * 8, 8)
        r3h = pl.multiple_of(i * 8 + 256, 8)
        e3 = pl.multiple_of(i * 16, 16)
        for j in range(14):
            emit(c3, j, e3, 8, ld(w332, j, r3, 8), ld(w332, 14 + j, r3, 8),
                 ld(w332, j, r3h, 8), ld(w332, 14 + j, r3h, 8))
        i4 = jnp.minimum(i, 27)
        r4 = pl.multiple_of(i4 * 32, 32)
        r4h = pl.multiple_of(i4 * 32 + 896, 32)
        e4 = pl.multiple_of(i4 * 64, 64)
        for n in range(4):
            emit(c4, n, e4, 32, ld(w432, n, r4, 32), ld(w432, 4 + n, r4, 32),
                 ld(w432, n, r4h, 32), ld(w432, 4 + n, r4h, 32))

    def a_part(xr, xup32, up):

        def prologue(stg):
            xu_cp = pltpu.make_async_copy(x_hbm.at[:, pl.ds(RIDE, UP)], x3.at[:, pl.ds(RIDE, UP)], sems.at[S_XU])

            def xr_cp(g):
                s0 = pl.multiple_of(g * 16, 16)
                return pltpu.make_async_copy(x_hbm.at[pl.ds(s0, 16), pl.ds(0, RIDE)],
                                             x3.at[pl.ds(s0, 16), pl.ds(0, RIDE)], sems.at[S_XR + g])
            srcs = [w.bitcast(U32) for w in (wq_hbm, wk_hbm, wv_hbm)]

            def w_cps(m, p, g):
                res = []
                for dd in range(2):
                    off = 16 * dd + 4 * g
                    if not isinstance(g, int):
                        off = pl.multiple_of(off, 4)
                    res.append(pltpu.make_async_copy(srcs[m].at[:, pl.ds(off, 4)],
                                                     stg.at[p, :, pl.ds(4 * dd, 4)],
                                                     sems.at[S_P + p * 2 + dd]))
                return res

            def wait(m, g):
                for cp in w_cps(m, 3 * g + m, g):
                    cp.wait()

            def relayout_rows(m, g, half):
                r0 = half * 256 if isinstance(half, int) else pl.multiple_of(half * 256, 256)
                ch = stg.at[3 * g + m, pl.ds(r0, 256)].reshape(2048, DH)
                for c in range(2):
                    for hp in range(4):
                        v = ch[pl.ds(c * 1024 + hp, 256, stride=4), :]
                        lo = v.astype(jnp.uint16)
                        hi = (v >> 16).astype(jnp.uint16)
                        w32s[m][G * g + 2 * hp, pl.ds(r0 + c * 128, 128), :] = pltpu.bitcast(lo, U32)
                        w32s[m][G * g + 2 * hp + 1, pl.ds(r0 + c * 128, 128), :] = pltpu.bitcast(hi, U32)

            def ln_ride(s0, n):
                for u in range(n):
                    xr[s0 + u] = _ln(x3[s0 + u, 0:RIDE, :].astype(F32)).astype(BF)

            def proj(m, g, j0, n):
                a = pltpu.bitcast(xup32[...], BF)
                for jj in range(n):
                    j = j0 + jj
                    h0 = G * g + 2 * j
                    w = pltpu.bitcast(jnp.concatenate([w32s[m][h0], w32s[m][h0 + 1]], axis=1), BF)
                    r = jnp.dot(a, w, preferred_element_type=F32)
                    r0 = r[:, 0:DH].reshape(NSEG, UP, DH)
                    r1 = r[:, DH:2 * DH].reshape(NSEG, UP, DH)
                    up[(G // 2) * (3 * g + m) + j] = jnp.concatenate([r0, r1], axis=1).astype(BF)

            xu_cp.start()

            def start_group(g, carry):
                for m in range(3):
                    for cp in w_cps(m, 3 * g + m, g):
                        cp.start()
                xr_cp(g).start()
                return carry
            lax.fori_loop(0, NG, start_group, 0)
            xu_cp.wait()
            def ln_up(c, carry):
                z = _ln(x3[pl.ds(c * 16, 16), RIDE:SEG, :].astype(F32).reshape(16 * UP, D))
                xup32[pl.ds(pl.multiple_of(c * 64, 64), 64), :] = pltpu.bitcast(z.astype(BF), U32)
                return carry
            lax.fori_loop(0, 4, ln_up, 0)
            wait(0, 0)

            def rl0(half, carry):
                relayout_rows(0, 0, half)
                return carry
            lax.fori_loop(0, 2, rl0, 0)

            def body(g, carry):
                gn = jnp.minimum(g + 1, NG - 1)

                def ph0(half, c):
                    proj(0, g, 2 * half, 1)

                    @pl.when(half == 0)
                    def _():
                        wait(1, g)
                    relayout_rows(1, g, half)
                    proj(0, g, 2 * half + 1, 1)
                    return c
                lax.fori_loop(0, 2, ph0, 0)
                wait(2, g)

                def ph1(half, c):
                    relayout_rows(2, g, half)
                    proj(1, g, 2 * half, 2)
                    return c
                lax.fori_loop(0, 2, ph1, 0)

                @pl.when(g < NG - 1)
                def _():
                    wait(0, gn)
                xr_cp(g).wait()

                def ph2(half, c):
                    ln_ride(g * 16 + half * 8, 8)
                    relayout_rows(0, gn, half)
                    proj(2, g, 2 * half, 2)
                    return c
                lax.fori_loop(0, 2, ph2, 0)

                @pl.when(g == 1)
                def _():
                    def st(j, c):
                        slab_copy(wo_hbm, wo, S_WO, j).start()
                        return c
                    lax.fori_loop(0, 8, st, 0)

                    def st3(j, c):
                        slab_copy(w3_hbm, w3, S_W3, j).start()
                        return c
                    lax.fori_loop(0, 28, st3, 0)

                    def st4(j, c):
                        slab_copy(w4_hbm, w4, S_W4, j).start()
                        return c
                    lax.fori_loop(0, 8, st4, 0)
                return carry

            lax.fori_loop(0, NG, body, 0)

        pl.run_scoped(prologue, pltpu.VMEM((3 * NG, D // 2, 8, DH), U32))
        pl.run_scoped(functools.partial(later, xr, up), *LATER_SHAPES)

    def later(xr, up, h3, oup, c3, c4):
        wait_all(wo, S_WO)
        wait_all(w3, S_W3)
        wait_all(w4, S_W4)

        R2 = 2 * (M + SEG)
        ri = lax.broadcasted_iota(jnp.int32, (R2, R2), 0)
        ci = lax.broadcasted_iota(jnp.int32, (R2, R2), 1)
        hr = jnp.where(ri < 64, ri >> 5, (ri - 64) >> 3)
        pr = jnp.where(ri < 64, ri & 31, 32 + (ri & 7))
        hc = jnp.where(ci < 64, ci >> 5, (ci - 64) >> 3)
        pc = jnp.where(ci < 64, ci & 31, 32 + (ci & 7))
        mask = (hr == hc) & ((pr < M) | (pr >= pc))

        def step(s, mem):
            a = jnp.concatenate([mem, xr[s].astype(F32)], axis=0).astype(BF)

            def proj(m, g):
                w = pltpu.bitcast(jnp.concatenate([w32s[m][g * G + i] for i in range(G)], axis=1), BF)
                r = jnp.dot(a, w, preferred_element_type=F32)
                return [r[:, i * DH:(i + 1) * DH] for i in range(G)]

            def cat(m, pair, x0, x1):
                u = up[(3 * (pair // (G // 2)) + m) * (G // 2) + pair % (G // 2), s].astype(F32)
                return jnp.concatenate([x0, x1, u], axis=0)

            def scores(q, k):
                sc = jnp.where(mask, _dot_nt(q, k.astype(BF)) * SCALE, -1e9)
                mx = jnp.max(sc, axis=-1, keepdims=True)
                e = jnp.exp(sc - mx)
                inv = pltpu.reciprocal(jnp.sum(e, axis=-1, keepdims=True), approx=False, full_range=False)
                return e.astype(BF), inv

            os_ = {}

            def pv(pair, v, e, inv, dep=None):
                if dep is not None:
                    z = jnp.minimum(jnp.abs(dep), 0.0)
                    v = v + jnp.concatenate([z] * 10, axis=0)
                o = jnp.dot(e, v.astype(BF), preferred_element_type=F32) * inv
                h0 = 2 * pair
                oup[s, :, h0 * DH:(h0 + 1) * DH] = o[64:72]
                oup[s, :, (h0 + 1) * DH:(h0 + 2) * DH] = o[72:80]
                os_[h0] = o[0:32]
                os_[h0 + 1] = o[32:64]

            parts = []

            def wo_part(ha, hb):
                oc = jnp.concatenate([os_[h] for h in range(ha, hb)], axis=1)
                parts.append(_dot(oc, _slabs(wo32, 8, ha * 64, hb * 64)))

            es, vs = {}, {}
            for g in range(NG):
                qs, ks, vv = proj(0, g), proj(1, g), proj(2, g)
                if g > 0:
                    for j in range(G // 2):
                        p = (g - 1) * (G // 2) + j
                        pv(p, vs[p], *es[p])
                for j in range(G // 2):
                    p = g * (G // 2) + j
                    es[p] = scores(cat(0, p, qs[2 * j], qs[2 * j + 1]), cat(1, p, ks[2 * j], ks[2 * j + 1]))
                    vs[p] = cat(2, p, vv[2 * j], vv[2 * j + 1])
                    if g < NG - 1:
                        vs[p] = vs[p].astype(BF)
            wo_part(0, 16)
            for j in range(G // 2):
                p = (NG - 1) * (G // 2) + j
                pv(p, vs[p], *es[p], dep=parts[0][0:8, 3 * DH:4 * DH])
            wo_part(16, 24)
            wo_part(24, 32)
            res = parts[0] + parts[1] + parts[2]
            h3[s, 0:RIDE, :] = x3[s, 0:RIDE, :].astype(F32) + res[M:]
            return res[:M]

        def slab_start(src, dst, sem, j, n):
            @pl.when(jnp.logical_and(j >= 0, j < n))
            def _():
                slab_copy(src, dst, sem, jnp.clip(j, 0, n - 1)).start()

        def two_steps(i, mem):
            slab_start(w1_hbm, w1, S_W1, i - 8, 8)
            slab_start(w2_hbm, w2, S_W2, i - 16, 8)
            combos(i, c3, c4)
            return step(2 * i + 1, step(2 * i, mem))

        lax.fori_loop(0, NSEG // 2, two_steps, mem0_ref[...].astype(F32))

        def b_scope(hn_buf, t_buf, o_buf):
            b1(h3, oup, hn_buf, t_buf)
            b2(h3, hn_buf, t_buf, o_buf, c3.bitcast(U32), c4.bitcast(U32))
        pl.run_scoped(b_scope, pltpu.VMEM((S, D), F32), pltpu.VMEM((S + 16, D), F32),
                      pltpu.VMEM((4, HB, D), BF))

    def b1(h3, oup, hn_buf, t_buf):
        wait_all(w1, S_W1)
        wait_all(w2, S_W2)
        t_buf[0:8, :] = jnp.zeros((8, D), F32)
        t_buf[8 + S:16 + S, :] = jnp.zeros((8, D), F32)
        nb = HB // SEG

        def fin(s0):
            o = oup[pl.ds(s0, nb)].reshape(nb * UP, H * DH)
            res = _dot(o, _slabs(wo32, 8)).reshape(nb, UP, D)
            h3[pl.ds(s0, nb), RIDE:SEG, :] = x3[pl.ds(s0, nb), RIDE:SEG, :].astype(F32) + res

        def lns(s0, r0):
            hn = _ln(h3[pl.ds(s0, nb)].reshape(HB, D))
            hn_buf[pl.ds(r0, HB), :] = hn
            return _ln(hn)

        def pass1(b, carry):
            sa = pl.multiple_of(b * 2 * nb, nb)
            sb = pl.multiple_of(b * 2 * nb + nb, nb)
            ra = pl.multiple_of(b * RB, HB)
            rb = pl.multiple_of(b * RB + HB, HB)
            fin(sa)
            fin(sb)
            za = lns(sa, ra)
            ya = _dot(za, _slabs(w132, 8))
            zb = lns(sb, rb)
            t_buf[pl.ds(ra + 8, HB), :] = _gelu(ya)
            yb = _dot(zb, _slabs(w132, 8))
            t_buf[pl.ds(rb + 8, HB), :] = _gelu(yb)
            return carry
        lax.fori_loop(0, S // RB, pass1, 0)

    def b2(h3, hn_buf, t_buf, o_buf, c3, c4):
        nb = HB // SEG

        def out_copy(hb, slot):
            return pltpu.make_async_copy(o_buf.at[slot], out_hbm.at[pl.ds(hb * HB, HB)], sems.at[S_OUT + slot])

        def pass2(b, carry):
            par = b % 2

            @pl.when(b >= 2)
            def _():
                out_copy(2 * b - 4, 2 * par).wait()
                out_copy(2 * b - 3, 2 * par + 1).wait()

            def shift(r0):
                parts = []
                for g, sh in enumerate((1, -1, 2, -2)):
                    tv = t_buf[pl.ds(r0, HB + 16), g * 256:(g + 1) * 256]
                    parts.append(tv[8 - sh:8 - sh + HB])
                return jnp.concatenate(parts, axis=1)

            def mix(r0, gm):
                x1 = hn_buf[pl.ds(r0, HB), :] + _dot(gm, _slabs(w232, 8))
                return x1, _ln(x1)

            def lhs7(a11, a12, a21, a22):
                return [a11 + a22, a21 + a22, a11, a22, a11 + a12, a21 - a11, a12 - a22]

            def comb(m):
                m1, m2, m3, m4, m5, m6, m7 = m
                return (m1 + m4 - m5 + m7, m3 + m5, m2 + m4, m1 - m2 + m3 + m6)

            def bf(v):
                return pltpu.bitcast(v, BF)

            ra = pl.multiple_of(b * RB, HB)
            rb = pl.multiple_of(b * RB + HB, HB)
            sa = pl.multiple_of(b * 2 * nb, nb)
            sb = pl.multiple_of(b * 2 * nb + nb, nb)
            ga = shift(ra)
            gb = shift(rb)
            xa, za = mix(ra, ga)
            xb, zb = mix(rb, gb)
            l3 = [v.astype(BF) for v in lhs7(za[:, :512], za[:, 512:], zb[:, :512], zb[:, 512:])]
            l4 = [[] for _ in range(7)]

            def rhs3(j):
                return [c3[0, j], w332[j, 0:256, :], c3[1, j], c3[2, j], w332[14 + j, 256:512, :],
                        c3[3, j], c3[4, j]]
            pre = {}
            for j in range(2):
                rhs = rhs3(j)
                for i in (2, 4):
                    pre[(i, j)] = _dot(l3[i], bf(rhs[i]))
            for j in range(14):
                rhs = rhs3(j)
                m = [pre[(i, j)] if (i, j) in pre else _dot(l3[i], bf(rhs[i])) for i in range(7)]
                u11, u12, u21, u22 = (_gelu(c) for c in comb(m))
                for i, v in enumerate(lhs7(u11, u12, u21, u22)):
                    l4[i].append(v)
            l4 = [jnp.concatenate(v, axis=1).astype(BF) for v in l4]
            hs = [(h3[pl.ds(sa, nb)].reshape(HB, D), xa), (h3[pl.ds(sb, nb)].reshape(HB, D), xb)]
            for n in range(4):
                rhs = [c4[0, n], w432[n, 0:896, :], c4[1, n], c4[2, n], w432[4 + n, 896:1792, :],
                       c4[3, n], c4[4, n]]
                m = [_dot(l4[i], bf(rhs[i])) for i in range(7)]
                h11, h12, h21, h22 = comb(m)
                for i, col, v in ((0, n, h11), (0, 4 + n, h12), (1, n, h21), (1, 4 + n, h22)):
                    cs = slice(col * 128, (col + 1) * 128)
                    res = hs[i][0][:, cs] + (hs[i][1][:, cs] + v)
                    o_buf[2 * par + i, :, cs] = res.astype(BF)
            out_copy(2 * b, 2 * par).start()
            out_copy(2 * b + 1, 2 * par + 1).start()
            return carry

        lax.fori_loop(0, S // RB, pass2, 0)
        for i in range(4):
            out_copy(S // HB - 4 + i, i).wait()

    LATER_SHAPES = (pltpu.VMEM((NSEG, SEG, D), F32), pltpu.VMEM((NSEG, UP, H * DH), F32),
                    pltpu.VMEM((5, 14, 512, 128), BF), pltpu.VMEM((5, 4, 1792, 128), BF))
    pl.run_scoped(
        a_part,
        pltpu.VMEM((NSEG, RIDE, D), BF),
        pltpu.VMEM((NSEG * UP // 2, D), U32),
        pltpu.VMEM((3 * H // 2, NSEG, 16, DH), BF),
    )


@jax.jit
def pallas_sequential_preLN__memory_aug_recurrent_mem_tr__mixer_s_mlp__prompt_kernel(A_x, A_mem0, A_Wq, A_Wk, A_Wv, A_Wo, A_seg_len, B_x, B_w1, B_w2, B_w3, B_w4):
    del A_seg_len, B_x
    any_spec = pl.BlockSpec(memory_space=pl.ANY)
    out = pl.pallas_call(
        _kernel,
        out_shape=jax.ShapeDtypeStruct((S, D), BF),
        in_specs=[any_spec, pl.BlockSpec(memory_space=pltpu.VMEM)] + [any_spec] * 8,
        out_specs=any_spec,
        scratch_shapes=[
            pltpu.VMEM((NSEG, SEG, D), BF),
            pltpu.VMEM((H, D // 2, DH), U32),
            pltpu.VMEM((H, D // 2, DH), U32),
            pltpu.VMEM((H, D // 2, DH), U32),
            pltpu.VMEM((8, H * DH, 128), BF),
            pltpu.VMEM((8, D, 128), BF),
            pltpu.VMEM((8, D, 128), BF),
            pltpu.VMEM((28, D, 128), BF),
            pltpu.VMEM((8, FF, 128), BF),
            pltpu.SemaphoreType.DMA((38,)),
        ],
        compiler_params=pltpu.CompilerParams(vmem_limit_bytes=127 * 1024 * 1024),
    )(
        A_x.reshape(NSEG, SEG, D), A_mem0.reshape(M, D),
        A_Wq.reshape(D // 2, 2 * H, DH), A_Wk.reshape(D // 2, 2 * H, DH), A_Wv.reshape(D // 2, 2 * H, DH),
        A_Wo.reshape(H * DH, D), B_w1, B_w2, B_w3, B_w4,
    )
    return out.reshape(1, S, D)
```

```python
import functools

import jax
import jax.numpy as jnp
import numpy as np
from jax import lax
import jax.experimental.pallas as pl
import jax.experimental.pallas.tpu as pltpu

BF = jnp.bfloat16
F32 = jnp.float32
U32 = jnp.uint32

S = 2048
D = 1024
H = 32
DH = 128
M = 8
SEG = 32
NSEG = S // SEG
FF = 3584
RIDE = 24
UP = SEG - RIDE
EPS = 1e-5
SCALE = DH ** -0.5
RB = 256
HB = RB // 2
G = 8
NG = H // G

def _ln(x):
    m = jnp.mean(x, axis=-1, keepdims=True)
    xc = x - m
    v = jnp.mean(xc * xc, axis=-1, keepdims=True)
    return xc * lax.rsqrt(v + EPS)


def _gelu(x):
    c0 = np.float32(np.sqrt(2.0 / np.pi))
    c1 = np.float32(np.sqrt(2.0 / np.pi) * 0.044715)
    t = jnp.tanh(x * (c0 + c1 * (x * x)))
    hx = 0.5 * x
    return hx + hx * t


def _dot(a, b):
    return jnp.dot(a.astype(BF), b, preferred_element_type=F32)


def _dot_nt(a, b):
    return lax.dot_general(a.astype(BF), b, (((1,), (1,)), ((), ())), preferred_element_type=F32)


def _slabs(w32, n, lo=None, hi=None):
    if lo is None:
        parts = [w32[j] for j in range(n)]
    else:
        parts = [w32[j, lo:hi, :] for j in range(n)]
    return pltpu.bitcast(jnp.concatenate(parts, axis=1), BF)


def _kernel(x_hbm, mem0_ref, wq_hbm, wk_hbm, wv_hbm, wo_hbm, w1_hbm, w2_hbm, w3_hbm, w4_hbm,
            out_hbm,
            x3, wq32, wk32, wv32, wo, w1, w2, w3, w4, sems):
    w32s = (wq32, wk32, wv32)
    wo32 = wo.bitcast(U32)
    w132, w232, w332, w432 = (w.bitcast(U32) for w in (w1, w2, w3, w4))
    S_XU, S_W1, S_W2, S_W3, S_W4, S_WO, S_OUT, S_XR, S_P = 0, 1, 2, 3, 4, 5, 6, 10, 14

    def slab_copy(src, dst, sem, j):
        j0 = j * 128 if isinstance(j, int) else pl.multiple_of(j * 128, 128)
        return pltpu.make_async_copy(src.at[:, pl.ds(j0, 128)], dst.at[j], sems.at[sem])

    def wait_all(buf, sem):
        pltpu.make_async_copy(buf, buf, sems.at[sem]).wait()

    def combos(i, c3, c4):
        def ld(ref, slab, r0, n):
            return pltpu.bitcast(ref[slab, pl.ds(r0, n), :], BF).astype(F32)

        def emit(dst, slab, e0, n, b11, b12, b21, b22):
            for i, v in enumerate((b11 + b22, b12 - b22, b21 - b11, b11 + b12, b21 + b22)):
                dst[i, slab, pl.ds(e0, 2 * n), :] = v.astype(BF)
        r3 = pl.multiple_of(i * 8, 8)
        r3h = pl.multiple_of(i * 8 + 256, 8)
        e3 = pl.multiple_of(i * 16, 16)
        for j in range(14):
            emit(c3, j, e3, 8, ld(w332, j, r3, 8), ld(w332, 14 + j, r3, 8),
                 ld(w332, j, r3h, 8), ld(w332, 14 + j, r3h, 8))
        i4 = jnp.minimum(i, 27)
        r4 = pl.multiple_of(i4 * 32, 32)
        r4h = pl.multiple_of(i4 * 32 + 896, 32)
        e4 = pl.multiple_of(i4 * 64, 64)
        for n in range(4):
            emit(c4, n, e4, 32, ld(w432, n, r4, 32), ld(w432, 4 + n, r4, 32),
                 ld(w432, n, r4h, 32), ld(w432, 4 + n, r4h, 32))

    def a_part(xr, xup32, up):

        def prologue(stg):
            xu_cp = pltpu.make_async_copy(x_hbm.at[:, pl.ds(RIDE, UP)], x3.at[:, pl.ds(RIDE, UP)], sems.at[S_XU])

            def xr_cp(g):
                s0 = pl.multiple_of(g * 16, 16)
                return pltpu.make_async_copy(x_hbm.at[pl.ds(s0, 16), pl.ds(0, RIDE)],
                                             x3.at[pl.ds(s0, 16), pl.ds(0, RIDE)], sems.at[S_XR + g])
            srcs = [w.bitcast(U32) for w in (wq_hbm, wk_hbm, wv_hbm)]

            def w_cps(m, p, g):
                res = []
                for dd in range(2):
                    off = 16 * dd + 4 * g
                    if not isinstance(g, int):
                        off = pl.multiple_of(off, 4)
                    res.append(pltpu.make_async_copy(srcs[m].at[:, pl.ds(off, 4)],
                                                     stg.at[p, :, pl.ds(4 * dd, 4)],
                                                     sems.at[S_P + p]))
                return res

            def wait(m, g):
                for cp in w_cps(m, 3 * g + m, g):
                    cp.wait()

            def relayout_rows(m, g, half):
                r0 = half * 256 if isinstance(half, int) else pl.multiple_of(half * 256, 256)
                ch = stg.at[3 * g + m, pl.ds(r0, 256)].reshape(2048, DH)
                for c in range(2):
                    for hp in range(4):
                        v = ch[pl.ds(c * 1024 + hp, 256, stride=4), :]
                        lo = v.astype(jnp.uint16)
                        hi = (v >> 16).astype(jnp.uint16)
                        w32s[m][G * g + 2 * hp, pl.ds(r0 + c * 128, 128), :] = pltpu.bitcast(lo, U32)
                        w32s[m][G * g + 2 * hp + 1, pl.ds(r0 + c * 128, 128), :] = pltpu.bitcast(hi, U32)

            def ln_ride(s0, n):
                for u in range(n):
                    xr[s0 + u] = _ln(x3[s0 + u, 0:RIDE, :].astype(F32)).astype(BF)

            def proj(m, g, j0, n):
                a = pltpu.bitcast(xup32[...], BF)
                for jj in range(n):
                    j = j0 + jj
                    h0 = G * g + 2 * j
                    w = pltpu.bitcast(jnp.concatenate([w32s[m][h0], w32s[m][h0 + 1]], axis=1), BF)
                    r = jnp.dot(a, w, preferred_element_type=F32)
                    r0 = r[:, 0:DH].reshape(NSEG, UP, DH)
                    r1 = r[:, DH:2 * DH].reshape(NSEG, UP, DH)
                    up[(G // 2) * (3 * g + m) + j] = jnp.concatenate([r0, r1], axis=1).astype(BF)

            xu_cp.start()

            def start_group(g, carry):
                for m in range(3):
                    for cp in w_cps(m, 3 * g + m, g):
                        cp.start()
                xr_cp(g).start()
                return carry
            lax.fori_loop(0, NG, start_group, 0)
            xu_cp.wait()
            def ln_up(c, carry):
                z = _ln(x3[pl.ds(c * 16, 16), RIDE:SEG, :].astype(F32).reshape(16 * UP, D))
                xup32[pl.ds(pl.multiple_of(c * 64, 64), 64), :] = pltpu.bitcast(z.astype(BF), U32)
                return carry
            lax.fori_loop(0, 4, ln_up, 0)
            wait(0, 0)

            def rl0(half, carry):
                relayout_rows(0, 0, half)
                return carry
            lax.fori_loop(0, 2, rl0, 0)

            def body(g, carry):
                gn = jnp.minimum(g + 1, NG - 1)

                def ph0(half, c):
                    proj(0, g, 2 * half, 1)

                    @pl.when(half == 0)
                    def _():
                        wait(1, g)
                    relayout_rows(1, g, half)
                    proj(0, g, 2 * half + 1, 1)
                    return c
                lax.fori_loop(0, 2, ph0, 0)
                wait(2, g)

                def ph1(half, c):
                    relayout_rows(2, g, half)
                    proj(1, g, 2 * half, 2)
                    return c
                lax.fori_loop(0, 2, ph1, 0)

                @pl.when(g < NG - 1)
                def _():
                    wait(0, gn)
                xr_cp(g).wait()

                def ph2(half, c):
                    ln_ride(g * 16 + half * 8, 8)
                    relayout_rows(0, gn, half)
                    proj(2, g, 2 * half, 2)
                    return c
                lax.fori_loop(0, 2, ph2, 0)

                @pl.when(g == 1)
                def _():
                    def st(j, c):
                        slab_copy(wo_hbm, wo, S_WO, j).start()
                        return c
                    lax.fori_loop(0, 8, st, 0)

                    def st3(j, c):
                        slab_copy(w3_hbm, w3, S_W3, j).start()
                        return c
                    lax.fori_loop(0, 28, st3, 0)

                    def st4(j, c):
                        slab_copy(w4_hbm, w4, S_W4, j).start()
                        return c
                    lax.fori_loop(0, 8, st4, 0)
                return carry

            lax.fori_loop(0, NG, body, 0)

        pl.run_scoped(prologue, pltpu.VMEM((3 * NG, D // 2, 8, DH), U32))
        pl.run_scoped(functools.partial(later, xr, up), *LATER_SHAPES)

    def later(xr, up, h3, oup, c3, c4):
        wait_all(wo, S_WO)
        wait_all(w3, S_W3)
        wait_all(w4, S_W4)

        R2 = 2 * (M + SEG)
        ri = lax.broadcasted_iota(jnp.int32, (R2, R2), 0)
        ci = lax.broadcasted_iota(jnp.int32, (R2, R2), 1)
        hr = jnp.where(ri < 64, ri >> 5, (ri - 64) >> 3)
        pr = jnp.where(ri < 64, ri & 31, 32 + (ri & 7))
        hc = jnp.where(ci < 64, ci >> 5, (ci - 64) >> 3)
        pc = jnp.where(ci < 64, ci & 31, 32 + (ci & 7))
        mask = (hr == hc) & ((pr < M) | (pr >= pc))

        def step(s, mem, extra=None):
            a = jnp.concatenate([mem, xr[s].astype(F32)], axis=0).astype(BF)

            def proj(m, g):
                w = pltpu.bitcast(jnp.concatenate([w32s[m][g * G + i] for i in range(G)], axis=1), BF)
                r = jnp.dot(a, w, preferred_element_type=F32)
                return [r[:, i * DH:(i + 1) * DH] for i in range(G)]

            def cat(m, pair, x0, x1):
                u = up[(3 * (pair // (G // 2)) + m) * (G // 2) + pair % (G // 2), s].astype(F32)
                return jnp.concatenate([x0, x1, u], axis=0)

            def scores(q, k):
                sc = jnp.where(mask, _dot_nt(q, k.astype(BF)) * SCALE, -1e9)
                mx = jnp.max(sc, axis=-1, keepdims=True)
                e = jnp.exp(sc - mx)
                inv = pltpu.reciprocal(jnp.sum(e, axis=-1, keepdims=True), approx=False, full_range=False)
                return e.astype(BF), inv

            os_ = {}

            def pv(pair, v, e, inv, dep=None):
                if dep is not None:
                    z = jnp.minimum(jnp.abs(dep), 0.0)
                    v = v + jnp.concatenate([z] * 10, axis=0)
                o = jnp.dot(e, v.astype(BF), preferred_element_type=F32) * inv
                h0 = 2 * pair
                oup[s, :, h0 * DH:(h0 + 1) * DH] = o[64:72]
                oup[s, :, (h0 + 1) * DH:(h0 + 2) * DH] = o[72:80]
                os_[h0] = o[0:32]
                os_[h0 + 1] = o[32:64]

            parts = []

            def wo_part(ha, hb):
                oc = jnp.concatenate([os_[h] for h in range(ha, hb)], axis=1)
                parts.append(_dot(oc, _slabs(wo32, 8, ha * 64, hb * 64)))

            es, vs = {}, {}
            for g in range(NG):
                qs, ks, vv = proj(0, g), proj(1, g), proj(2, g)
                if g > 0:
                    for j in range(G // 2):
                        p = (g - 1) * (G // 2) + j
                        pv(p, vs[p], *es[p])
                for j in range(G // 2):
                    p = g * (G // 2) + j
                    es[p] = scores(cat(0, p, qs[2 * j], qs[2 * j + 1]), cat(1, p, ks[2 * j], ks[2 * j + 1]))
                    vs[p] = cat(2, p, vv[2 * j], vv[2 * j + 1])
                    if g < NG - 1:
                        vs[p] = vs[p].astype(BF)
            wo_part(0, 16)
            dep = parts[0][0:8, 5 * DH:6 * DH]
            if extra is not None:
                dep = dep + extra
            for j in range(G // 2):
                p = (NG - 1) * (G // 2) + j
                pv(p, vs[p], *es[p], dep=dep)
            wo_part(16, 24)
            wo_part(24, 32)
            res = parts[0] + parts[1] + parts[2]
            h3[s, 0:RIDE, :] = x3[s, 0:RIDE, :].astype(F32) + res[M:]
            return res[:M]

        def slab_start(src, dst, sem, j, n):
            @pl.when(jnp.logical_and(j >= 0, j < n))
            def _():
                slab_copy(src, dst, sem, jnp.clip(j, 0, n - 1)).start()

        def two_steps(i, mem):
            slab_start(w1_hbm, w1, S_W1, i - 8, 8)
            slab_start(w2_hbm, w2, S_W2, i - 16, 8)
            combos(i, c3, c4)
            e3 = pl.multiple_of(i * 16, 16)
            e4 = pl.multiple_of(jnp.minimum(i, 27) * 64, 64)
            ex = c3[4, 13, pl.ds(e3, 16), :].astype(F32)[0:8] + c4[4, 3, pl.ds(e4, 16), :].astype(F32)[0:8]
            return step(2 * i + 1, step(2 * i, mem, ex))

        lax.fori_loop(0, NSEG // 2, two_steps, mem0_ref[...].astype(F32))

        def b_scope(hn_buf, t_buf, o_buf):
            b1(h3, oup, hn_buf, t_buf)
            b2(h3, hn_buf, t_buf, o_buf, c3.bitcast(U32), c4.bitcast(U32))
        pl.run_scoped(b_scope, pltpu.VMEM((S, D), F32), pltpu.VMEM((S + 16, D), F32),
                      pltpu.VMEM((4, HB, D), BF))

    def b1(h3, oup, hn_buf, t_buf):
        wait_all(w1, S_W1)
        wait_all(w2, S_W2)
        t_buf[0:8, :] = jnp.zeros((8, D), F32)
        t_buf[8 + S:16 + S, :] = jnp.zeros((8, D), F32)
        nb = HB // SEG

        def fin(s0):
            o = oup[pl.ds(s0, nb)].reshape(nb * UP, H * DH)
            res = _dot(o, _slabs(wo32, 8)).reshape(nb, UP, D)
            h3[pl.ds(s0, nb), RIDE:SEG, :] = x3[pl.ds(s0, nb), RIDE:SEG, :].astype(F32) + res

        def lns(s0, r0):
            hn = _ln(h3[pl.ds(s0, nb)].reshape(HB, D))
            hn_buf[pl.ds(r0, HB), :] = hn
            return _ln(hn)

        def pass1(b, carry):
            sa = pl.multiple_of(b * 2 * nb, nb)
            sb = pl.multiple_of(b * 2 * nb + nb, nb)
            ra = pl.multiple_of(b * RB, HB)
            rb = pl.multiple_of(b * RB + HB, HB)
            fin(sa)
            fin(sb)
            za = lns(sa, ra)
            ya = _dot(za, _slabs(w132, 8))
            zb = lns(sb, rb)
            t_buf[pl.ds(ra + 8, HB), :] = _gelu(ya)
            yb = _dot(zb, _slabs(w132, 8))
            t_buf[pl.ds(rb + 8, HB), :] = _gelu(yb)
            return carry
        lax.fori_loop(0, S // RB, pass1, 0)

    def b2(h3, hn_buf, t_buf, o_buf, c3, c4):
        nb = HB // SEG

        def out_copy(hb, slot):
            return pltpu.make_async_copy(o_buf.at[slot], out_hbm.at[pl.ds(hb * HB, HB)], sems.at[S_OUT + slot])

        def pass2(b, carry):
            par = b % 2

            @pl.when(b >= 2)
            def _():
                out_copy(2 * b - 4, 2 * par).wait()
                out_copy(2 * b - 3, 2 * par + 1).wait()

            def shift(r0):
                parts = []
                for g, sh in enumerate((1, -1, 2, -2)):
                    tv = t_buf[pl.ds(r0, HB + 16), g * 256:(g + 1) * 256]
                    parts.append(tv[8 - sh:8 - sh + HB])
                return jnp.concatenate(parts, axis=1)

            def mix(r0, gm):
                x1 = hn_buf[pl.ds(r0, HB), :] + _dot(gm, _slabs(w232, 8))
                return x1, _ln(x1)

            def lhs7(a11, a12, a21, a22):
                return [a11 + a22, a21 + a22, a11, a22, a11 + a12, a21 - a11, a12 - a22]

            def comb(m):
                m1, m2, m3, m4, m5, m6, m7 = m
                return (m1 + m4 - m5 + m7, m3 + m5, m2 + m4, m1 - m2 + m3 + m6)

            def bf(v):
                return pltpu.bitcast(v, BF)

            ra = pl.multiple_of(b * RB, HB)
            rb = pl.multiple_of(b * RB + HB, HB)
            sa = pl.multiple_of(b * 2 * nb, nb)
            sb = pl.multiple_of(b * 2 * nb + nb, nb)
            ga = shift(ra)
            gb = shift(rb)
            xa, za = mix(ra, ga)
            xb, zb = mix(rb, gb)
            l3 = [v.astype(BF) for v in lhs7(za[:, :512], za[:, 512:], zb[:, :512], zb[:, 512:])]
            l4 = [[] for _ in range(7)]

            def rhs3(j):
                return [c3[0, j], w332[j, 0:256, :], c3[1, j], c3[2, j], w332[14 + j, 256:512, :],
                        c3[3, j], c3[4, j]]
            pre = {}
            for j in range(2):
                rhs = rhs3(j)
                for i in (2, 4):
                    pre[(i, j)] = _dot(l3[i], bf(rhs[i]))
            for j in range(14):
                rhs = rhs3(j)
                m = [pre[(i, j)] if (i, j) in pre else _dot(l3[i], bf(rhs[i])) for i in range(7)]
                u11, u12, u21, u22 = (_gelu(c) for c in comb(m))
                for i, v in enumerate(lhs7(u11, u12, u21, u22)):
                    l4[i].append(v)
            l4 = [jnp.concatenate(v, axis=1).astype(BF) for v in l4]
            hs = [(h3[pl.ds(sa, nb)].reshape(HB, D), xa), (h3[pl.ds(sb, nb)].reshape(HB, D), xb)]
            for n in range(4):
                rhs = [c4[0, n], w432[n, 0:896, :], c4[1, n], c4[2, n], w432[4 + n, 896:1792, :],
                       c4[3, n], c4[4, n]]
                m = [_dot(l4[i], bf(rhs[i])) for i in range(7)]
                h11, h12, h21, h22 = comb(m)
                for i, col, v in ((0, n, h11), (0, 4 + n, h12), (1, n, h21), (1, 4 + n, h22)):
                    cs = slice(col * 128, (col + 1) * 128)
                    res = hs[i][0][:, cs] + (hs[i][1][:, cs] + v)
                    o_buf[2 * par + i, :, cs] = res.astype(BF)
            out_copy(2 * b, 2 * par).start()
            out_copy(2 * b + 1, 2 * par + 1).start()
            return carry

        lax.fori_loop(0, S // RB, pass2, 0)
        for i in range(4):
            out_copy(S // HB - 4 + i, i).wait()

    LATER_SHAPES = (pltpu.VMEM((NSEG, SEG, D), F32), pltpu.VMEM((NSEG, UP, H * DH), F32),
                    pltpu.VMEM((5, 14, 512, 128), BF), pltpu.VMEM((5, 4, 1792, 128), BF))
    pl.run_scoped(
        a_part,
        pltpu.VMEM((NSEG, RIDE, D), BF),
        pltpu.VMEM((NSEG * UP // 2, D), U32),
        pltpu.VMEM((3 * H // 2, NSEG, 16, DH), BF),
    )


@jax.jit
def pallas_sequential_preLN__memory_aug_recurrent_mem_tr__mixer_s_mlp__prompt_kernel(A_x, A_mem0, A_Wq, A_Wk, A_Wv, A_Wo, A_seg_len, B_x, B_w1, B_w2, B_w3, B_w4):
    del A_seg_len, B_x
    any_spec = pl.BlockSpec(memory_space=pl.ANY)
    out = pl.pallas_call(
        _kernel,
        out_shape=jax.ShapeDtypeStruct((S, D), BF),
        in_specs=[any_spec, pl.BlockSpec(memory_space=pltpu.VMEM)] + [any_spec] * 8,
        out_specs=any_spec,
        scratch_shapes=[
            pltpu.VMEM((NSEG, SEG, D), BF),
            pltpu.VMEM((H, D // 2, DH), U32),
            pltpu.VMEM((H, D // 2, DH), U32),
            pltpu.VMEM((H, D // 2, DH), U32),
            pltpu.VMEM((8, H * DH, 128), BF),
            pltpu.VMEM((8, D, 128), BF),
            pltpu.VMEM((8, D, 128), BF),
            pltpu.VMEM((28, D, 128), BF),
            pltpu.VMEM((8, FF, 128), BF),
            pltpu.SemaphoreType.DMA((26,)),
        ],
        compiler_params=pltpu.CompilerParams(
            vmem_limit_bytes=127 * 1024 * 1024,
            flags={"XLA_TPU_RESCHEDULE_DMA_DONES": True}),
    )(
        A_x.reshape(NSEG, SEG, D), A_mem0.reshape(M, D),
        A_Wq.reshape(D // 2, 2 * H, DH), A_Wk.reshape(D // 2, 2 * H, DH), A_Wv.reshape(D // 2, 2 * H, DH),
        A_Wo.reshape(H * DH, D), B_w1, B_w2, B_w3, B_w4,
    )
    return out.reshape(1, S, D)
```

```python
import functools

import jax
import jax.numpy as jnp
import numpy as np
from jax import lax
import jax.experimental.pallas as pl
import jax.experimental.pallas.tpu as pltpu

BF = jnp.bfloat16
F32 = jnp.float32
U32 = jnp.uint32

S = 2048
D = 1024
H = 32
DH = 128
M = 8
SEG = 32
NSEG = S // SEG
FF = 3584
RIDE = 24
UP = SEG - RIDE
EPS = 1e-5
SCALE = DH ** -0.5
RB = 256
HB = RB // 2
G = 8
NG = H // G

def _ln(x):
    m = jnp.mean(x, axis=-1, keepdims=True)
    xc = x - m
    v = jnp.mean(xc * xc, axis=-1, keepdims=True)
    return xc * lax.rsqrt(v + EPS)


def _gelu(x):
    c0 = np.float32(np.sqrt(2.0 / np.pi))
    c1 = np.float32(np.sqrt(2.0 / np.pi) * 0.044715)
    t = jnp.tanh(x * (c0 + c1 * (x * x)))
    hx = 0.5 * x
    return hx + hx * t


def _dot(a, b):
    return jnp.dot(a.astype(BF), b, preferred_element_type=F32)


def _dot_nt(a, b):
    return lax.dot_general(a.astype(BF), b, (((1,), (1,)), ((), ())), preferred_element_type=F32)


def _slabs(w32, n, lo=None, hi=None):
    if lo is None:
        parts = [w32[j] for j in range(n)]
    else:
        parts = [w32[j, lo:hi, :] for j in range(n)]
    return pltpu.bitcast(jnp.concatenate(parts, axis=1), BF)


def _kernel(x_hbm, mem0_ref, wq_hbm, wk_hbm, wv_hbm, wo_hbm, w1_hbm, w2_hbm, w3_hbm, w4_hbm,
            out_hbm,
            x3, wq32, wk32, wv32, wo, w1, w2, w3, w4, sems):
    w32s = (wq32, wk32, wv32)
    wo32 = wo.bitcast(U32)
    w132, w232, w332, w432 = (w.bitcast(U32) for w in (w1, w2, w3, w4))
    S_XU, S_W1, S_W2, S_W3, S_W4, S_WO, S_OUT, S_XR, S_P = 0, 1, 2, 3, 4, 5, 6, 10, 14

    def slab_copy(src, dst, sem, j):
        j0 = j * 128 if isinstance(j, int) else pl.multiple_of(j * 128, 128)
        return pltpu.make_async_copy(src.at[:, pl.ds(j0, 128)], dst.at[j], sems.at[sem])

    def wait_all(buf, sem):
        pltpu.make_async_copy(buf, buf, sems.at[sem]).wait()

    def combos(i, c3, c4):
        def ld(ref, slab, r0, n):
            return pltpu.bitcast(ref[slab, pl.ds(r0, n), :], BF).astype(F32)

        def emit(dst, slab, e0, n, b11, b12, b21, b22):
            for i, v in enumerate((b11 + b22, b12 - b22, b21 - b11, b11 + b12, b21 + b22)):
                dst[i, slab, pl.ds(e0, 2 * n), :] = v.astype(BF)
        r3 = pl.multiple_of(i * 8, 8)
        r3h = pl.multiple_of(i * 8 + 256, 8)
        e3 = pl.multiple_of(i * 16, 16)
        for j in range(14):
            emit(c3, j, e3, 8, ld(w332, j, r3, 8), ld(w332, 14 + j, r3, 8),
                 ld(w332, j, r3h, 8), ld(w332, 14 + j, r3h, 8))
        i4 = jnp.minimum(i, 27)
        r4 = pl.multiple_of(i4 * 32, 32)
        r4h = pl.multiple_of(i4 * 32 + 896, 32)
        e4 = pl.multiple_of(i4 * 64, 64)
        for n in range(4):
            emit(c4, n, e4, 32, ld(w432, n, r4, 32), ld(w432, 4 + n, r4, 32),
                 ld(w432, n, r4h, 32), ld(w432, 4 + n, r4h, 32))

    def a_part(xr, xup32, up):

        def prologue(stg):
            xu_cp = pltpu.make_async_copy(x_hbm.at[:, pl.ds(RIDE, UP)], x3.at[:, pl.ds(RIDE, UP)], sems.at[S_XU])

            def xr_cp(g):
                s0 = pl.multiple_of(g * 16, 16)
                return pltpu.make_async_copy(x_hbm.at[pl.ds(s0, 16), pl.ds(0, RIDE)],
                                             x3.at[pl.ds(s0, 16), pl.ds(0, RIDE)], sems.at[S_XR + g])
            srcs = [w.bitcast(U32) for w in (wq_hbm, wk_hbm, wv_hbm)]

            def w_cps(m, p, g):
                res = []
                for dd in range(2):
                    off = 16 * dd + 4 * g
                    if not isinstance(g, int):
                        off = pl.multiple_of(off, 4)
                    res.append(pltpu.make_async_copy(srcs[m].at[:, pl.ds(off, 4)],
                                                     stg.at[p, :, pl.ds(4 * dd, 4)],
                                                     sems.at[S_P + p]))
                return res

            def wait(m, g):
                for cp in w_cps(m, 3 * g + m, g):
                    cp.wait()

            def relayout_rows(m, g, half):
                r0 = half * 256 if isinstance(half, int) else pl.multiple_of(half * 256, 256)
                ch = stg.at[3 * g + m, pl.ds(r0, 256)].reshape(2048, DH)
                for c in range(2):
                    for hp in range(4):
                        v = ch[pl.ds(c * 1024 + hp, 256, stride=4), :]
                        lo = v.astype(jnp.uint16)
                        hi = (v >> 16).astype(jnp.uint16)
                        w32s[m][G * g + 2 * hp, pl.ds(r0 + c * 128, 128), :] = pltpu.bitcast(lo, U32)
                        w32s[m][G * g + 2 * hp + 1, pl.ds(r0 + c * 128, 128), :] = pltpu.bitcast(hi, U32)

            def ln_ride(s0, n):
                for u in range(n):
                    xr[s0 + u] = _ln(x3[s0 + u, 0:RIDE, :].astype(F32)).astype(BF)

            def proj(m, g, j0, n):
                a = pltpu.bitcast(xup32[...], BF)
                for jj in range(n):
                    j = j0 + jj
                    h0 = G * g + 2 * j
                    w = pltpu.bitcast(jnp.concatenate([w32s[m][h0], w32s[m][h0 + 1]], axis=1), BF)
                    r = jnp.dot(a, w, preferred_element_type=F32)
                    r0 = r[:, 0:DH].reshape(NSEG, UP, DH)
                    r1 = r[:, DH:2 * DH].reshape(NSEG, UP, DH)
                    up[(G // 2) * (3 * g + m) + j] = jnp.concatenate([r0, r1], axis=1).astype(BF)

            xu_cp.start()

            def start_group(g, carry):
                for m in range(3):
                    for cp in w_cps(m, 3 * g + m, g):
                        cp.start()
                xr_cp(g).start()
                return carry
            lax.fori_loop(0, NG, start_group, 0)
            xu_cp.wait()
            def ln_up(c, carry):
                z = _ln(x3[pl.ds(c * 16, 16), RIDE:SEG, :].astype(F32).reshape(16 * UP, D))
                xup32[pl.ds(pl.multiple_of(c * 64, 64), 64), :] = pltpu.bitcast(z.astype(BF), U32)
                return carry
            lax.fori_loop(0, 4, ln_up, 0)
            wait(0, 0)

            def rl0(half, carry):
                relayout_rows(0, 0, half)
                return carry
            lax.fori_loop(0, 2, rl0, 0)

            def body(g, carry):
                gn = jnp.minimum(g + 1, NG - 1)

                def ph0(half, c):
                    proj(0, g, 2 * half, 1)

                    @pl.when(half == 0)
                    def _():
                        wait(1, g)
                    relayout_rows(1, g, half)
                    proj(0, g, 2 * half + 1, 1)
                    return c
                lax.fori_loop(0, 2, ph0, 0)
                wait(2, g)

                def ph1(half, c):
                    relayout_rows(2, g, half)
                    proj(1, g, 2 * half, 2)
                    return c
                lax.fori_loop(0, 2, ph1, 0)

                @pl.when(g < NG - 1)
                def _():
                    wait(0, gn)
                xr_cp(g).wait()

                def ph2(half, c):
                    ln_ride(g * 16 + half * 8, 8)
                    relayout_rows(0, gn, half)
                    proj(2, g, 2 * half, 2)
                    return c
                lax.fori_loop(0, 2, ph2, 0)

                @pl.when(g == 1)
                def _():
                    def st(j, c):
                        slab_copy(wo_hbm, wo, S_WO, j).start()
                        return c
                    lax.fori_loop(0, 8, st, 0)

                    def st3(j, c):
                        slab_copy(w3_hbm, w3, S_W3, j).start()
                        return c
                    lax.fori_loop(0, 28, st3, 0)

                    def st4(j, c):
                        slab_copy(w4_hbm, w4, S_W4, j).start()
                        return c
                    lax.fori_loop(0, 8, st4, 0)
                return carry

            lax.fori_loop(0, NG, body, 0)

        pl.run_scoped(prologue, pltpu.VMEM((3 * NG, D // 2, 8, DH), U32))
        pl.run_scoped(functools.partial(later, xr, up), *LATER_SHAPES)

    def later(xr, up, h3, oup, c3, c4):
        wait_all(wo, S_WO)
        wait_all(w3, S_W3)
        wait_all(w4, S_W4)

        R2 = 2 * (M + SEG)
        ri = lax.broadcasted_iota(jnp.int32, (R2, R2), 0)
        ci = lax.broadcasted_iota(jnp.int32, (R2, R2), 1)
        hr = jnp.where(ri < 64, ri >> 5, (ri - 64) >> 3)
        pr = jnp.where(ri < 64, ri & 31, 32 + (ri & 7))
        hc = jnp.where(ci < 64, ci >> 5, (ci - 64) >> 3)
        pc = jnp.where(ci < 64, ci & 31, 32 + (ci & 7))
        mask = (hr == hc) & ((pr < M) | (pr >= pc))

        def step(s, mem):
            a = jnp.concatenate([mem, xr[s].astype(F32)], axis=0).astype(BF)

            def proj(m, g):
                w = pltpu.bitcast(jnp.concatenate([w32s[m][g * G + i] for i in range(G)], axis=1), BF)
                r = jnp.dot(a, w, preferred_element_type=F32)
                return [r[:, i * DH:(i + 1) * DH] for i in range(G)]

            def cat(m, pair, x0, x1):
                u = up[(3 * (pair // (G // 2)) + m) * (G // 2) + pair % (G // 2), s].astype(F32)
                return jnp.concatenate([x0, x1, u], axis=0)

            def scores(q, k):
                sc = jnp.where(mask, _dot_nt(q, k.astype(BF)) * SCALE, -1e9)
                mx = jnp.max(sc, axis=-1, keepdims=True)
                e = jnp.exp(sc - mx)
                inv = pltpu.reciprocal(jnp.sum(e, axis=-1, keepdims=True), approx=False, full_range=False)
                return e.astype(BF), inv

            os_ = {}

            def pv(pair, v, e, inv, dep=None):
                if dep is not None:
                    z = jnp.minimum(jnp.abs(dep), 0.0)
                    v = v + jnp.concatenate([z] * 10, axis=0)
                o = jnp.dot(e, v.astype(BF), preferred_element_type=F32) * inv
                h0 = 2 * pair
                oup[s, :, h0 * DH:(h0 + 1) * DH] = o[64:72]
                oup[s, :, (h0 + 1) * DH:(h0 + 2) * DH] = o[72:80]
                os_[h0] = o[0:32]
                os_[h0 + 1] = o[32:64]

            parts = []

            def wo_part(ha, hb):
                oc = jnp.concatenate([os_[h] for h in range(ha, hb)], axis=1)
                parts.append(_dot(oc, _slabs(wo32, 8, ha * 64, hb * 64)))

            es, vs = {}, {}
            for g in range(NG):
                qs, ks, vv = proj(0, g), proj(1, g), proj(2, g)
                if g > 0:
                    for j in range(G // 2):
                        p = (g - 1) * (G // 2) + j
                        pv(p, vs[p], *es[p])
                for j in range(G // 2):
                    p = g * (G // 2) + j
                    es[p] = scores(cat(0, p, qs[2 * j], qs[2 * j + 1]), cat(1, p, ks[2 * j], ks[2 * j + 1]))
                    vs[p] = cat(2, p, vv[2 * j], vv[2 * j + 1])
                    if g < NG - 1:
                        vs[p] = vs[p].astype(BF)
            wo_part(0, 16)
            dep = parts[0][0:8, 5 * DH:6 * DH]
            for j in range(G // 2):
                p = (NG - 1) * (G // 2) + j
                pv(p, vs[p], *es[p], dep=dep)
            wo_part(16, 25)
            wo_part(25, 32)
            res = parts[0] + parts[1] + parts[2]
            h3[s, 0:RIDE, :] = x3[s, 0:RIDE, :].astype(F32) + res[M:]
            return res[:M]

        def slab_start(src, dst, sem, j, n):
            @pl.when(jnp.logical_and(j >= 0, j < n))
            def _():
                slab_copy(src, dst, sem, jnp.clip(j, 0, n - 1)).start()

        def two_steps(i, mem):
            slab_start(w1_hbm, w1, S_W1, i - 8, 8)
            slab_start(w2_hbm, w2, S_W2, i - 16, 8)
            combos(i, c3, c4)
            e3 = pl.multiple_of(i * 16, 16)
            e4 = pl.multiple_of(jnp.minimum(i, 27) * 64, 64)
            ex = c3[4, 13, pl.ds(e3, 16), :].astype(F32)[0:8] + c4[4, 3, pl.ds(e4, 16), :].astype(F32)[0:8]
            z = jnp.minimum(jnp.abs(ex), 0.0)
            m2 = step(2 * i + 1, step(2 * i, mem))
            return jnp.concatenate([m2[:, 0:7 * DH], m2[:, 7 * DH:] + z], axis=1)

        lax.fori_loop(0, NSEG // 2, two_steps, mem0_ref[...].astype(F32))

        def b_scope(hn_buf, t_buf, o_buf):
            b1(h3, oup, hn_buf, t_buf)
            b2(h3, hn_buf, t_buf, o_buf, c3.bitcast(U32), c4.bitcast(U32))
        pl.run_scoped(b_scope, pltpu.VMEM((S, D), F32), pltpu.VMEM((S + 16, D), F32),
                      pltpu.VMEM((4, HB, D), BF))

    def b1(h3, oup, hn_buf, t_buf):
        wait_all(w1, S_W1)
        wait_all(w2, S_W2)
        t_buf[0:8, :] = jnp.zeros((8, D), F32)
        t_buf[8 + S:16 + S, :] = jnp.zeros((8, D), F32)
        nb = HB // SEG

        def fin(s0):
            o = oup[pl.ds(s0, nb)].reshape(nb * UP, H * DH)
            res = _dot(o, _slabs(wo32, 8)).reshape(nb, UP, D)
            h3[pl.ds(s0, nb), RIDE:SEG, :] = x3[pl.ds(s0, nb), RIDE:SEG, :].astype(F32) + res

        def lns(s0, r0):
            hn = _ln(h3[pl.ds(s0, nb)].reshape(HB, D))
            hn_buf[pl.ds(r0, HB), :] = hn
            return _ln(hn)

        def pass1(b, carry):
            sa = pl.multiple_of(b * 2 * nb, nb)
            sb = pl.multiple_of(b * 2 * nb + nb, nb)
            ra = pl.multiple_of(b * RB, HB)
            rb = pl.multiple_of(b * RB + HB, HB)
            fin(sa)
            fin(sb)
            za = lns(sa, ra)
            ya = _dot(za, _slabs(w132, 8))
            zb = lns(sb, rb)
            t_buf[pl.ds(ra + 8, HB), :] = _gelu(ya)
            yb = _dot(zb, _slabs(w132, 8))
            t_buf[pl.ds(rb + 8, HB), :] = _gelu(yb)
            return carry
        lax.fori_loop(0, S // RB, pass1, 0)

    def b2(h3, hn_buf, t_buf, o_buf, c3, c4):
        nb = HB // SEG

        def out_copy(hb, slot):
            return pltpu.make_async_copy(o_buf.at[slot], out_hbm.at[pl.ds(hb * HB, HB)], sems.at[S_OUT + slot])

        def pass2(b, carry):
            par = b % 2

            @pl.when(b >= 2)
            def _():
                out_copy(2 * b - 4, 2 * par).wait()
                out_copy(2 * b - 3, 2 * par + 1).wait()

            def shift(r0):
                parts = []
                for g, sh in enumerate((1, -1, 2, -2)):
                    tv = t_buf[pl.ds(r0, HB + 16), g * 256:(g + 1) * 256]
                    parts.append(tv[8 - sh:8 - sh + HB])
                return jnp.concatenate(parts, axis=1)

            def mix(r0, gm):
                x1 = hn_buf[pl.ds(r0, HB), :] + _dot(gm, _slabs(w232, 8))
                return x1, _ln(x1)

            def lhs7(a11, a12, a21, a22):
                return [a11 + a22, a21 + a22, a11, a22, a11 + a12, a21 - a11, a12 - a22]

            def comb(m):
                m1, m2, m3, m4, m5, m6, m7 = m
                return (m1 + m4 - m5 + m7, m3 + m5, m2 + m4, m1 - m2 + m3 + m6)

            def bf(v):
                return pltpu.bitcast(v, BF)

            ra = pl.multiple_of(b * RB, HB)
            rb = pl.multiple_of(b * RB + HB, HB)
            sa = pl.multiple_of(b * 2 * nb, nb)
            sb = pl.multiple_of(b * 2 * nb + nb, nb)
            ga = shift(ra)
            gb = shift(rb)
            xa, za = mix(ra, ga)
            xb, zb = mix(rb, gb)
            l3 = [v.astype(BF) for v in lhs7(za[:, :512], za[:, 512:], zb[:, :512], zb[:, 512:])]
            l4 = [[] for _ in range(7)]

            def rhs3(j):
                return [c3[0, j], w332[j, 0:256, :], c3[1, j], c3[2, j], w332[14 + j, 256:512, :],
                        c3[3, j], c3[4, j]]
            pre = {}
            for j in range(2):
                rhs = rhs3(j)
                for i in (2, 4):
                    pre[(i, j)] = _dot(l3[i], bf(rhs[i]))
            for j in range(14):
                rhs = rhs3(j)
                m = [pre[(i, j)] if (i, j) in pre else _dot(l3[i], bf(rhs[i])) for i in range(7)]
                u11, u12, u21, u22 = (_gelu(c) for c in comb(m))
                for i, v in enumerate(lhs7(u11, u12, u21, u22)):
                    l4[i].append(v)
            l4 = [jnp.concatenate(v, axis=1).astype(BF) for v in l4]
            hs = [(h3[pl.ds(sa, nb)].reshape(HB, D), xa), (h3[pl.ds(sb, nb)].reshape(HB, D), xb)]
            for n in range(4):
                rhs = [c4[0, n], w432[n, 0:896, :], c4[1, n], c4[2, n], w432[4 + n, 896:1792, :],
                       c4[3, n], c4[4, n]]
                m = [_dot(l4[i], bf(rhs[i])) for i in range(7)]
                h11, h12, h21, h22 = comb(m)
                for i, col, v in ((0, n, h11), (0, 4 + n, h12), (1, n, h21), (1, 4 + n, h22)):
                    cs = slice(col * 128, (col + 1) * 128)
                    res = hs[i][0][:, cs] + (hs[i][1][:, cs] + v)
                    o_buf[2 * par + i, :, cs] = res.astype(BF)
            out_copy(2 * b, 2 * par).start()
            out_copy(2 * b + 1, 2 * par + 1).start()
            return carry

        lax.fori_loop(0, S // RB, pass2, 0)
        for i in range(4):
            out_copy(S // HB - 4 + i, i).wait()

    LATER_SHAPES = (pltpu.VMEM((NSEG, SEG, D), F32), pltpu.VMEM((NSEG, UP, H * DH), F32),
                    pltpu.VMEM((5, 14, 512, 128), BF), pltpu.VMEM((5, 4, 1792, 128), BF))
    pl.run_scoped(
        a_part,
        pltpu.VMEM((NSEG, RIDE, D), BF),
        pltpu.VMEM((NSEG * UP // 2, D), U32),
        pltpu.VMEM((3 * H // 2, NSEG, 16, DH), BF),
    )


@jax.jit
def pallas_sequential_preLN__memory_aug_recurrent_mem_tr__mixer_s_mlp__prompt_kernel(A_x, A_mem0, A_Wq, A_Wk, A_Wv, A_Wo, A_seg_len, B_x, B_w1, B_w2, B_w3, B_w4):
    del A_seg_len, B_x
    any_spec = pl.BlockSpec(memory_space=pl.ANY)
    out = pl.pallas_call(
        _kernel,
        out_shape=jax.ShapeDtypeStruct((S, D), BF),
        in_specs=[any_spec, pl.BlockSpec(memory_space=pltpu.VMEM)] + [any_spec] * 8,
        out_specs=any_spec,
        scratch_shapes=[
            pltpu.VMEM((NSEG, SEG, D), BF),
            pltpu.VMEM((H, D // 2, DH), U32),
            pltpu.VMEM((H, D // 2, DH), U32),
            pltpu.VMEM((H, D // 2, DH), U32),
            pltpu.VMEM((8, H * DH, 128), BF),
            pltpu.VMEM((8, D, 128), BF),
            pltpu.VMEM((8, D, 128), BF),
            pltpu.VMEM((28, D, 128), BF),
            pltpu.VMEM((8, FF, 128), BF),
            pltpu.SemaphoreType.DMA((26,)),
        ],
        compiler_params=pltpu.CompilerParams(
            vmem_limit_bytes=127 * 1024 * 1024,
            flags={"XLA_TPU_RESCHEDULE_DMA_DONES": True}),
    )(
        A_x.reshape(NSEG, SEG, D), A_mem0.reshape(M, D),
        A_Wq.reshape(D // 2, 2 * H, DH), A_Wk.reshape(D // 2, 2 * H, DH), A_Wv.reshape(D // 2, 2 * H, DH),
        A_Wo.reshape(H * DH, D), B_w1, B_w2, B_w3, B_w4,
    )
    return out.reshape(1, S, D)
```
